```python
import jax
import jax.numpy as jnp

def _softmax(x, axis=-1):
    return jax.nn.softmax(x, axis=axis)
def _gelu(x):
    return jax.nn.gelu(x, approximate=True)
def _silu(x):
    return jax.nn.silu(x)
def _sigmoid(x):
    return jax.nn.sigmoid(x)
def _layernorm(x, axis=-1, eps=1e-5):
    m = jnp.mean(x, axis=axis, keepdims=True)
    v = jnp.var(x, axis=axis, keepdims=True)
    return (x - m) / jnp.sqrt(v + eps)
def _scatter_add(tgt, idx, src, axis=0):
    return tgt.at[idx].add(src)
def _segment_sum(src, seg, n):
    return jax.ops.segment_sum(src, seg, n)
class _Rng:
    def __init__(self, key):
        self._k = key
    def _next(self):
        self._k, sub = jax.random.split(self._k)
        return sub
    def normal(self, shape):
        return jax.random.normal(self._next(), shape, dtype=jnp.bfloat16)
    def randint(self, lo, hi, shape):
        return jax.random.randint(self._next(), shape, lo, hi, dtype=jnp.int32)
    def uniform(self, shape, lo=0.0, hi=1.0):
        return jax.random.uniform(self._next(), shape, jnp.bfloat16, lo, hi)
    def permutation(self, n):
        return jax.random.permutation(self._next(), n)


kernel_name = 'gated_mix__sliding_block_cached__moe_arch_mod__decode'

def setup_inputs():
    _rng = _Rng(jax.random.key(int.from_bytes(__import__("os").urandom(4), "little")))
    _w = (lambda a: (lambda t: t.astype(jnp.bfloat16) if jnp.issubdtype(t.dtype, jnp.floating) else t)(jnp.asarray(a)))
    def _A_setup():
        B, Sq, D = 1, 1, 640
        Hq, Hkv, Sk, Dh = 32, 32, 32768, 192
        assert Hq % Hkv == 0, (Hq, Hkv)
        return {
            "x": _w((lambda *s: _rng.normal(s) * 0.05)(B, Sq, D)),
            "k_cache": _w((lambda *s: _rng.normal(s) * 0.05)(B, Hkv, Sk, Dh)),
            "v_cache": _w((lambda *s: _rng.normal(s) * 0.05)(B, Hkv, Sk, Dh)),
            "wq": _w((lambda *s: _rng.normal(s) * 0.05)(D, Hq * Dh) * (D ** -0.5)),
            "wo": _w((lambda *s: _rng.normal(s) * 0.05)(Hq * Dh, D) * ((Hq * Dh) ** -0.5)),
        }
    _A_in = _A_setup()

    def _B_setup():
        B, S, D, F, C = 1, 1, 640, 1536, 1
        return {
            "x": _w((lambda *s: _rng.normal(s) * 0.05)(B, S, D)),
            "w_r": _w((lambda *s: _rng.normal(s) * 0.05)(D)),
            "w_gate": _w((lambda *s: _rng.normal(s) * 0.05)(D, F)),
            "w_up": _w((lambda *s: _rng.normal(s) * 0.05)(D, F)),
            "w_down": _w((lambda *s: _rng.normal(s) * 0.05)(F, D)),
        }
    _B_in = _B_setup()

    return {
        "A_x": _A_in["x"],
        "A_k_cache": _A_in["k_cache"],
        "A_v_cache": _A_in["v_cache"],
        "A_wq": _A_in["wq"],
        "A_wo": _A_in["wo"],
        "B_x": _B_in["x"],
        "B_w_r": _B_in["w_r"],
        "B_w_gate": _B_in["w_gate"],
        "B_w_up": _B_in["w_up"],
        "B_w_down": _B_in["w_down"],
        "gate_w": _w((lambda *s: _rng.normal(s) * 0.05)(640)),
    }

def reference(A_x, A_k_cache, A_v_cache, A_wq, A_wo, B_x, B_w_r, B_w_gate, B_w_up, B_w_down, gate_w):
    def _A_ref(x, k_cache, v_cache, wq, wo):
        B, Sq, D = x.shape
        Hq, Dh = 32, 192
        Hkv, Sk = k_cache.shape[1], k_cache.shape[2]
        W = min(4096, max(256, Sk // 4))
        rep = Hq // Hkv
        q = (lambda x, *d: x.transpose(*d))((x @ wq).reshape(B, Sq, Hq, Dh), 0, 2, 1, 3)
        k = jnp.repeat(k_cache[:, :, Sk - W:, :], rep, axis=1)
        v = jnp.repeat(v_cache[:, :, Sk - W:, :], rep, axis=1)
        scores = jnp.einsum("bhqd,bhkd->bhqk", q, k) * (Dh ** -0.5)
        p = _softmax(scores, axis=-1)
        o = jnp.einsum("bhqk,bhkd->bhqd", p, v)
        return (lambda x, *d: x.transpose(*d))(o, 0, 2, 1, 3).reshape(B, Sq, Hq * Dh) @ wo

    def _B_ref(x, w_r, w_gate, w_up, w_down):
        B, S, D = x.shape
        C = 1
        r = x @ w_r
        idx = jnp.argsort(-r, axis=-1)[:, :C]
        idx_e = jnp.repeat(idx.reshape(B, C, 1), D, axis=2)
        x_sel = jnp.take_along_axis(x, idx_e, axis=1)
        g = _silu(x_sel @ w_gate)
        u = x_sel @ w_up
        y = (g * u) @ w_down
        r_sel = _sigmoid(jnp.take_along_axis(r, idx, axis=1))
        y = y * r_sel.reshape(B, C, 1)
        b_off = (jnp.arange(B) * S).reshape(B, 1)
        flat_idx = (idx + b_off).reshape(B * C)
        zero = (x * 0.0).reshape(B * S, D)
        upd = _scatter_add(zero, flat_idx, y.reshape(B * C, D), axis=0)
        return x + upd.reshape(B, S, D)

    x = A_x
    g = _sigmoid((x * gate_w).sum(-1, keepdims=True))
    a = _A_ref(x, A_k_cache, A_v_cache, A_wq, A_wo)
    b = _B_ref(x, B_w_r, B_w_gate, B_w_up, B_w_down)
    return g * a + (1 - g) * b
```

```python
import functools

import jax
import jax.numpy as jnp
import jax.experimental.pallas as pl
import jax.experimental.pallas.tpu as pltpu

H, DH, SK, D, F = 32, 192, 32768, 640, 1536
W = min(4096, max(256, SK // 4))
BASE = SK - W
NP = H // 2
PR = 2 * DH

REG, RW = 15, 128
GW = 8
NG = RW // GW

f32 = jnp.float32
bf16 = jnp.bfloat16


def _iota(shape, dim):
    return jax.lax.broadcasted_iota(jnp.int32, shape, dim)


def _interleave(*lists):
    items = []
    for n, lst in enumerate(lists):
        items += [((i + 0.5) / len(lst), n, v) for i, v in enumerate(lst)]
    return [v for _, _, v in sorted(items, key=lambda t: t[:2])]


def _kernel(x_hbm, kT, vT, wq, wo, wr_hbm, wg, wu, wd, gw_hbm, out_ref,
            x_v, wr_v, gw_v, wq_b, k_b, v_b, wo_b, wg_b, wu_b, wd_b,
            q_s, o_s, oe_s, ob_s, mix_s, s_s, p_s,
            sems, *, cfg):
    LOOK, LAG, SWEEP, NB = cfg['look'], cfg['lag'], cfg['sweep'], cfg['nb']
    copy = pltpu.make_async_copy

    class Sems:
        def __init__(self, first):
            self.first, self.at = first, self

        def __getitem__(self, i):
            return sems.at[self.first + i]

    sm_sem, k_sem, v_sem, f_sem, wo_sem, last_sem = (Sems(n) for n in (1, 4, 6, 8, 11, 11 + NG))
    wq_sem = sems.at[0]

    def rows(base, r0, n):
        r = base + r0
        return pl.ds(r if isinstance(r, int) else pl.multiple_of(r, 8), n)

    def region_piece(src, dst, sem, r, nr, c, nc):
        idx = (pl.ds(r, nr), pl.ds(c, nc))
        return lambda: copy(src.at[idx], dst.at[idx], sem)

    def alternate(pieces, solo=0):
        return [(pc, 1 if i % 2 or i >= len(pieces) - solo else 0) for i, pc in enumerate(pieces)]

    sweep = [(r, c) for c in range(0, RW, 2) for r in range(0, REG, 3)]
    n_last = len(sweep) // NG
    wq_pieces = alternate([region_piece(wq, wq_b, wq_sem, r, 3, c, 2) for r, c in sweep])
    wo_pieces = alternate(
        [region_piece(wo, wo_b, wo_sem.at[c // GW], r, 3, c, 2) for r, c in sweep[:-n_last]]
        + [region_piece(wo, wo_b, last_sem.at[i // cfg['lg']], r, 3, c, 2) for i, (r, c) in enumerate(sweep[-n_last:])],
        LOOK)

    NF = cfg['nf']

    def pair_pieces(p, with_ffn):
        slot = p % 2

        def kv(src, buf, sem, r0, c):
            return lambda: copy(src.at[rows(p * PR, r0, 8 * NB), pl.ds(BASE + c, 512)],
                                buf.at[slot, pl.ds(r0, 8 * NB), pl.ds(c, 512)], sem.at[slot])

        def ffn(src, dst, k, r0, n):
            def make():
                idx = rows(p * (src.shape[0] // NF), r0, n)
                return copy(src.at[idx], dst.at[idx], f_sem.at[k])
            return make

        cache = [kv(src, buf, sem, g + r, c)
                 for src, buf, sem in ((kT, k_b, k_sem), (vT, v_b, v_sem))
                 for g in range(0, PR, 8 * SWEEP)
                 for c in range(0, W, 512) for r in range(0, 8 * SWEEP, 8 * NB)]
        if not with_ffn:
            return alternate(cache)
        small = _interleave([ffn(wg, wg_b, 0, r, 8) for r in range(0, D // NF, 8)],
                            [ffn(wu, wu_b, 1, r, 8) for r in range(0, D // NF, 8)],
                            [ffn(wd, wd_b, 2, r, 16) for r in range(0, F // NF, 16)])
        return alternate(_interleave(cache, small))

    def stream(cur, nxt, tasks):
        ahead = [pc for pc, queue in cur + nxt if queue == 1][LOOK:]
        n = 0
        for i, (pc, queue) in enumerate(cur):
            if queue == 0:
                pc().start(priority=0)
            else:
                if n < len(ahead):
                    ahead[n]().start(priority=1)
                n += 1
            for fn in tasks.get(i, ()):
                if cfg.get('scopes'):
                    with jax.named_scope(f"xs{i}"):
                        fn()
                else:
                    fn()

    def spread(tasks, first, step, fns):
        for n, fn in enumerate(fns):
            tasks.setdefault(first + n * step, []).append(fn)

    st = {}
    small_copies = [copy(x_hbm, x_v, sm_sem.at[0]), copy(gw_hbm, gw_v, sm_sem.at[1]),
                    copy(wr_hbm, wr_v, sm_sem.at[2])]

    def expand_x():
        for c in small_copies:
            c.wait()
        x = x_v[0].astype(f32)
        nb = D // 8
        own = _iota((nb, D), 1) // 8 == _iota((nb, D), 0)
        rep = _iota((D, 128), 0) % 8 == _iota((D, 128), 1) % 8
        oe_s[0:nb] = jnp.dot(jnp.where(own, x, 0.0).astype(bf16), jnp.where(rep, 1.0, 0.0).astype(bf16),
                             preferred_element_type=f32)

    def q_slice(r):
        def fn():
            if r == 0:
                copy(wq_b, wq_b, wq_sem).wait()
                st['q'] = [jnp.zeros((16, 128), f32)] * 3
            diag = _iota((16, 128), 1) // 8 == _iota((16, 128), 0)
            for g in range(NG):
                band, m = divmod(r * NG + g, 3)
                lhs = jnp.where(diag, oe_s[band:band + 1], 0.0).astype(bf16)
                rhs = wq_b[r, g * GW:(g + 1) * GW].reshape(128, 128)
                st['q'][m] = st['q'][m] + jnp.dot(lhs, rhs, preferred_element_type=f32)
            if r == REG - 1:
                for m in range(3):
                    q_s[16 * m:16 * (m + 1)] = st['q'][m]
        return fn

    def own_head():
        return (_iota((8, PR), 1) >= DH) == (_iota((8, PR), 0) % 2 == 1)

    def qk_slices(p, n=4):
        cw = W // n

        def part(j):
            def fn():
                if j == 0:
                    buf = k_b.at[p % 2]
                    copy(buf, buf, k_sem.at[p % 2]).wait()
                    q = jnp.concatenate([q_s[pl.ds(3 * p + m, 1)] for m in range(3)], axis=1)
                    st['lhs'] = jnp.where(own_head(), q, 0.0).astype(bf16)
                sl = slice(j * cw, (j + 1) * cw)
                s_s[:, sl] = jnp.dot(st['lhs'], k_b[p % 2, :, sl], preferred_element_type=f32)
            return fn

        def softmax():
            sc = s_s[...] * DH ** -0.5
            e = jnp.exp(sc - jnp.max(sc, axis=-1, keepdims=True))
            p_s[...] = e / jnp.sum(e, axis=-1, keepdims=True)

        return [part(j) for j in range(n)] + [softmax]

    def pv_slices(p, n=4):
        cw = W // n

        def part(j):
            def fn():
                if j == 0:
                    buf = v_b.at[p % 2]
                    copy(buf, buf, v_sem.at[p % 2]).wait()
                sl = slice(j * cw, (j + 1) * cw)
                o = jax.lax.dot_general(p_s[:, sl].astype(bf16), v_b[p % 2, :, sl],
                                        (((1,), (1,)), ((), ())), preferred_element_type=f32)
                st['o'] = o if j == 0 else st['o'] + o
                if j == n - 1:
                    o = jnp.where(_iota((1, PR), 1) < DH, st['o'][0:1], st['o'][1:2])
                    for m in range(3):
                        o_s[pl.ds(3 * p + m, 1)] = o[:, 128 * m:128 * (m + 1)]
            return fn

        return [part(j) for j in range(n)]

    last_bands = sorted({t // 5 for r in range(REG) for t in range(2 * (RW * (r + 1) - GW), 2 * RW * (r + 1))})

    def expand_o():
        o = o_s[...].astype(bf16)
        src, lane = _iota((128, 128), 0), _iota((128, 128), 1)
        for s in range(5):
            tile = 16 * s + lane // 8
            sel = (tile >= 5 * (src // 8)) & (tile < 5 * (src // 8) + 5) & (src % 8 == lane % 8)
            oe_s[48 * s:48 * (s + 1)] = jnp.dot(o, jnp.where(sel, 1.0, 0.0).astype(bf16),
                                                preferred_element_type=f32)
        tile = _iota((8, 128), 1) // 8
        st['col'] = [(16 * s + tile) % 5 == _iota((8, 128), 0) for s in range(5)]
        st['a'] = jnp.zeros((8, 128), f32)
        lane, row = _iota((8, 128), 1), _iota((8, 128), 0)
        lhs = jnp.concatenate([jnp.where(lane == 8 * (b % 16) + row, o_s[b // 16:b // 16 + 1], 0.0)
                               for b in last_bands], axis=0)
        ob_s[...] = jnp.dot(lhs.astype(bf16), jnp.ones((128, 128), bf16),
                            preferred_element_type=f32) * mix_s[8:9]

    def wo_block(r, g):
        a, s = divmod(r * NG + g, 5)
        lhs = jnp.where(st['col'][s], oe_s[48 * s + a:48 * s + a + 1], 0.0).astype(bf16)
        rhs = wo_b[r, g * GW:(g + 1) * GW].reshape(128, 128)
        st['a'] = st['a'] + jnp.dot(lhs, rhs, preferred_element_type=f32)

    def wo_slice(g):
        def fn():
            buf = wo_b.at[:, g * GW:(g + 1) * GW]
            copy(buf, buf, wo_sem.at[g]).wait()
            for r in range(REG):
                wo_block(r, g)
        return fn

    def ffn_slices():
        def up(k, buf):
            def fn():
                copy(buf, buf, f_sem.at[k]).wait()
                st[k] = jnp.dot(jnp.broadcast_to(x_v[0], (8, D)), buf[...], preferred_element_type=f32)
            return fn

        def down():
            copy(wd_b, wd_b, f_sem.at[2]).wait()
            h = (jax.nn.silu(st[0]) * st[1]).astype(bf16)
            y = jnp.dot(h, wd_b[...], preferred_element_type=f32)
            x = x_v[0].astype(f32)
            gate = jax.nn.sigmoid(jnp.sum(x * gw_v[...].astype(f32).reshape(1, D), axis=-1, keepdims=True))
            rsel = jax.nn.sigmoid(jnp.sum(x * wr_v[...].astype(f32).reshape(1, D), axis=-1, keepdims=True))
            b = (1.0 - gate) * (x + (x * 0.0 + y * rsel))
            folded = jnp.zeros((8, 128), f32)
            for m in range(D // 128):
                folded = jnp.where(_iota((8, 128), 0) == m, b[:, 128 * m:128 * (m + 1)], folded)
            mix_s[0:8] = folded
            mix_s[8:16] = jnp.broadcast_to(gate, (8, 128))

        return [up(0, wg_b), up(1, wu_b), down]

    wq_pieces[0][0]().start(priority=0)
    for pc, _ in wq_pieces[1:2 * LOOK:2]:
        pc().start(priority=1)
    stream(wq_pieces[1:], pair_pieces(0, True), {21: [c.start for c in small_copies], 21 + LAG: [expand_x]})

    def pair(p, with_ffn, nxt, before=None, extra=()):
        cur = pair_pieces(p, with_ffn)
        tasks = {}
        spread(tasks, 8, 24, extra)
        if before:
            spread(tasks, LAG, 6, before)
        else:
            spread(tasks, LAG, cfg['step'], pv_slices(p - 1, cfg['n']))
        spread(tasks, len(cur) // 2 + LAG, cfg['step'], qk_slices(p, cfg['n']))
        assert max(tasks) < len(cur)
        stream(cur, nxt, tasks)

    def pairs(lo, hi, with_ffn):
        def body(p, carry):
            pair(p, with_ffn, pair_pieces(p + 1, with_ffn))
            return carry
        jax.lax.fori_loop(lo, hi, body, 0)

    pair(0, True, pair_pieces(1, True), before=[q_slice(r) for r in range(REG)])
    pairs(1, NF - 1, True)
    pair(NF - 1, True, pair_pieces(NF, False))
    pairs(NF, NP - 1, False)
    pair(NP - 1, False, wo_pieces, extra=ffn_slices())

    tasks = {}
    spread(tasks, LAG, 10, pv_slices(NP - 1) + [expand_o])
    late = []
    pos = LAG + 50
    for g in range(NG - 1):
        pos = max(pos + 8, n_last * (g + 1) + LAG)
        if pos < len(wo_pieces) - LOOK:
            tasks.setdefault(pos, []).append(wo_slice(g))
        else:
            late.append(wo_slice(g))
    stream(wo_pieces, [], tasks)
    for fn in late:
        fn()

    rest = mix_s[8:16] * st['a'] + mix_s[0:8]
    row = _iota((8, 128), 0)
    acc = [jnp.where(row == m, rest, 0.0) for m in range(5)]
    for i0 in range(0, n_last, cfg['lg']):
        for i in range(i0, i0 + cfg['lg']):
            wo_pieces[i - n_last][0]().wait()
        for i in range(i0, i0 + cfg['lg']):
            r0, c0 = sweep[i - n_last]
            for r in range(r0, r0 + 3):
                for c in range(c0, c0 + 2):
                    w = wo_b[r, c].astype(f32)
                    for half in range(2):
                        band, m = divmod(2 * (RW * r + c) + half, 5)
                        k = last_bands.index(band)
                        acc[m] = acc[m] + w[8 * half:8 * half + 8] * ob_s[8 * k:8 * k + 8]
    out = jnp.concatenate([jnp.sum(a, axis=0, keepdims=True) for a in acc], axis=1)
    out_ref[0] = out.astype(bf16)


def _regions(w):
    r, c = w.shape
    return w.reshape(r // 8, 8, c // 128, 128).transpose(0, 2, 1, 3).reshape(REG, RW, 16, 128)


def make(**kw):
    cfg = dict(look=26, lag=55, sweep=24, nb=4, n=4, step=10, nf=8, lg=1)
    cfg.update(kw)

    def fn(A_x, A_k_cache, A_v_cache, A_wq, A_wo, B_x, B_w_r, B_w_gate, B_w_up, B_w_down, gate_w):
        del B_x
        kT = jnp.swapaxes(A_k_cache, 2, 3).reshape(H * DH, SK)
        vT = jnp.swapaxes(A_v_cache, 2, 3).reshape(H * DH, SK)
        any_spec = pl.BlockSpec(memory_space=pl.ANY)
        vmem, dma = pltpu.VMEM, pltpu.SemaphoreType.DMA
        return pl.pallas_call(
            functools.partial(_kernel, cfg=cfg),
            out_shape=jax.ShapeDtypeStruct((1, 1, D), bf16),
            in_specs=[any_spec] * 10,
            out_specs=pl.BlockSpec(memory_space=pltpu.VMEM),
            scratch_shapes=[
                vmem((1, 1, D), bf16), vmem((D,), bf16), vmem((D,), bf16),
                vmem((REG, RW, 16, 128), bf16), vmem((2, PR, W), bf16), vmem((2, PR, W), bf16),
                vmem((REG, RW, 16, 128), bf16), vmem((D, F), bf16), vmem((D, F), bf16), vmem((F, D), bf16),
                vmem((48, 128), f32), vmem((48, 128), f32), vmem((240, 128), f32), vmem((480, 128), f32), vmem((16, 128), f32),
                vmem((8, W), f32), vmem((8, W), f32),
                dma((11 + NG + 20,)),
            ],
            compiler_params=pltpu.CompilerParams(
                vmem_limit_bytes=64 * 1024 * 1024,
                disable_bounds_checks=True,
                disable_semaphore_checks=True,
            ),
            name="gated_mix_decode",
        )(A_x, kT, vT, _regions(A_wq), _regions(A_wo), B_w_r, B_w_gate, B_w_up, B_w_down, gate_w)
    return fn


pallas_gated_mix__sliding_block_cached__moe_arch_mod__decode_kernel = jax.jit(make())
```

```python
import functools

import jax
import jax.numpy as jnp
import jax.experimental.pallas as pl
import jax.experimental.pallas.tpu as pltpu

H, DH, SK, D, F = 32, 192, 32768, 640, 1536
W = min(4096, max(256, SK // 4))
BASE = SK - W
NP = H // 2
PR = 2 * DH

ROW, SEG = 256, 8
CT = D // 128
NG = ROW // 16
WO_ROWS, WD_ROWS = H * DH * D // 1024 // ROW, F * D // 1024 // ROW
TAIL0, TAIL1 = WD_ROWS * ROW, F * D // 1024

S_X, S_WQ, S_WG, S_WU, S_K, S_V, S_OUT, S_TAIL = 0, 3, 4, 5, 6, 8, 10, 10 + 2 * NG

f32 = jnp.float32
bf16 = jnp.bfloat16


def _iota(shape, dim):
    return jax.lax.broadcasted_iota(jnp.int32, shape, dim)


def _kernel(x_hbm, kT, vT, wq, wo, wr_hbm, wg, wu, wd, gw_hbm, out_ref,
            x_v, wr_v, gw_v, wq_b, k_b, v_b, wo_b, wg_b, wu_b, wd_b,
            q_s, oh_s, ex_s, hb_s, mix_s, s_s, p_s, sems, *, cfg):
    LOOK, LAG = cfg['look'], cfg['lag']

    def copy(src, dst, sem):
        return pltpu.make_async_copy(src, dst, sems.at[sem])

    def matrix_segment(src, dst, sem, t):
        nct, pieces, end = src.shape[1] // 128, [], t + SEG
        while t < end:
            band, c = divmod(t, nct)
            n = min(nct - c, end - t)
            idx = (pl.ds(8 * band, 8), pl.ds(128 * c, 128 * n))
            pieces.append(functools.partial(copy, src.at[idx], dst.at[idx], sem))
            t += n
        return pieces

    def flat_segment(src, dst, sem, t, n=SEG):
        idx = pl.ds(t // 2, n // 2)
        return [functools.partial(copy, src.at[idx], dst.at[idx], sem)]

    def queued(segments, period):
        return [(pc, 1 if i % period else 0) for i, seg in enumerate(segments) for pc in seg]

    NS = cfg['ns']
    first = queued(
        [matrix_segment(wq, wq_b, S_WQ, ROW + t) for t in range(0, NS, SEG)] +
        [matrix_segment(src, dst, sem, r * ROW + t)
         for parity in range(2) for t in range(0, ROW, SEG)
         for src, dst, sem in ((wq, wq_b, S_WQ), (wg, wg_b, S_WG), (wu, wu_b, S_WU))
         for r in range(parity, 15, 2)
         if (r * ROW + t) * 1024 < src.shape[0] * src.shape[1] and not (src is wq and r == 1 and t < NS)],
        cfg['pa'])

    last = queued(
        [flat_segment(src, dst, S_OUT + 2 * (t // 16) + k, r * ROW + t)
         for t in range(0, ROW, SEG) for parity in range(2)
         for k, (src, dst, n) in enumerate(((wo, wo_b, WO_ROWS), (wd, wd_b, WD_ROWS)))
         for r in range(parity, n, 2)],
        cfg['pc'])
    n_group = len(last) // NG
    TS, TL, TG = cfg['ts'], cfg['tl'], cfg['tg']
    solo = TAIL1 - TL * LOOK
    cuts = list(range(TAIL0, solo, TS)) + list(range(solo, TAIL1 + 1, TL))
    tail = [(a, b, S_TAIL + (a - TAIL0) // TG) for a, b in zip(cuts, cuts[1:])]
    last += [(flat_segment(wd, wd_b, sem, a, b - a)[0], 1 if a >= solo or (a - TAIL0) % 32 >= 8 else 0)
             for a, b, sem in tail]

    def pair_pieces(p):
        def piece(src, buf, sem, r, n, parity, c):
            def make():
                rows = pl.ds(8 * parity, 8)
                return copy(src.at[pl.ds(p * (PR // 16) + r, n), rows, pl.ds(BASE + c, 128 * SEG)],
                            buf.at[p % 2, pl.ds(r, n), rows, pl.ds(c, 128 * SEG)], sem + p % 2)
            return make

        n0, n1 = cfg['kv']
        cols = list(range(0, W, 128 * SEG))
        return [(piece(src, buf, sem, h + r + d, n, parity, c), queue)
                for src, buf, sem in ((kT, k_b, S_K), (vT, v_b, S_V))
                for h in (0, DH // 16) for parity in range(2) for c in (cols[::-1] if parity else cols)
                for r in range(0, DH // 16, n0 + n1) for d, n, queue in ((0, n0, 0), (n0, n1, 1))]

    def stream(cur, nxt, tasks):
        ahead = [pc for pc, queue in cur + nxt if queue == 1][LOOK:]
        n = 0
        for i, (pc, queue) in enumerate(cur):
            if queue == 0:
                pc().start(priority=0)
            else:
                if n < len(ahead):
                    ahead[n]().start(priority=1)
                n += 1
            for fn in tasks.get(i, ()):
                if cfg.get('scopes'):
                    with jax.named_scope(f"xs{i}"):
                        fn()
                else:
                    fn()

    def spread(tasks, start, step, fns):
        for n, fn in enumerate(fns):
            tasks.setdefault(start + n * step, []).append(fn)

    st = {}
    small_copies = [copy(x_hbm, x_v, S_X), copy(gw_hbm, gw_v, S_X + 1), copy(wr_hbm, wr_v, S_X + 2)]

    def fold(v, rows):
        folded = jnp.zeros((rows, 128), f32)
        for m in range(v.shape[1] // 128):
            folded = jnp.where(_iota((rows, 128), 0) == m, v[0:1, 128 * m:128 * (m + 1)], folded)
        return folded

    def gates():
        for c in small_copies:
            c.wait()
        x = x_v[0].astype(f32)
        gate = jax.nn.sigmoid(jnp.sum(x * gw_v[...].astype(f32).reshape(1, D), axis=-1, keepdims=True))
        rsel = jax.nn.sigmoid(jnp.sum(x * wr_v[...].astype(f32).reshape(1, D), axis=-1, keepdims=True))
        mix_s[0] = fold(x, 8)
        mix_s[1] = jnp.broadcast_to(gate, (8, 128))
        mix_s[2] = jnp.broadcast_to(rsel, (8, 128))

    def x_dot(w):
        return jnp.dot(jnp.broadcast_to(x_v[0], (8, D)), w, preferred_element_type=f32)

    def q_slice(p):
        def fn():
            if p == 0:
                copy(wq_b, wq_b, S_WQ).wait()
            q_s[p] = x_dot(wq_b[:, p * PR:(p + 1) * PR])
        return fn

    def hidden_slices():
        def gate_proj():
            copy(wg_b, wg_b, S_WG).wait()
            st['g'] = x_dot(wg_b[...])

        def up_proj():
            copy(wu_b, wu_b, S_WU).wait()
            oh_s[48:64] = fold(jax.nn.silu(st['g']) * x_dot(wu_b[...]), 16)

        return [gate_proj, up_proj]

    def cache_tile(buf, p, sl):
        return buf[p % 2, :, :, sl].reshape(PR, sl.stop - sl.start)

    def qk_slices(p, n=4):
        def part(j):
            def fn():
                if j == 0:
                    copy(k_b.at[p % 2], k_b.at[p % 2], S_K + p % 2).wait()
                    own = (_iota((8, PR), 1) >= DH) == (_iota((8, PR), 0) % 2 == 1)
                    st['q'] = jnp.where(own, q_s[p], 0.0).astype(bf16)
                sl = slice(j * W // n, (j + 1) * W // n)
                s_s[:, sl] = jnp.dot(st['q'], cache_tile(k_b, p, sl), preferred_element_type=f32)
            return fn

        def softmax():
            sc = s_s[...] * DH ** -0.5
            e = jnp.exp(sc - jnp.max(sc, axis=-1, keepdims=True))
            p_s[...] = e / jnp.sum(e, axis=-1, keepdims=True)

        return [part(j) for j in range(n)] + [softmax]

    def pv_slices(p, n=4):
        def part(j):
            def fn():
                if j == 0:
                    copy(v_b.at[p % 2], v_b.at[p % 2], S_V + p % 2).wait()
                sl = slice(j * W // n, (j + 1) * W // n)
                o = jax.lax.dot_general(p_s[:, sl].astype(bf16), cache_tile(v_b, p, sl),
                                        (((1,), (1,)), ((), ())), preferred_element_type=f32)
                st['o'] = o if j == 0 else st['o'] + o
                if j == n - 1:
                    o = jnp.where(_iota((1, PR), 1) < DH, st['o'][0:1], st['o'][1:2])
                    for m in range(PR // 128):
                        oh_s[pl.ds(PR // 128 * p + m, 1)] = o[:, 128 * m:128 * (m + 1)]
            return fn

        return [part(j) for j in range(n)]

    tail_bands = range(TAIL0 // CT, TAIL1 // CT)

    def expand():
        oh = oh_s[...].astype(bf16)
        src, lane = _iota((128, 128), 0), _iota((128, 128), 1)
        for s in range(CT):
            tile = 16 * s + lane // 8 - CT * (src // 8)
            sel = (tile >= 0) & (tile < CT) & (src % 8 == lane % 8)
            ex_s[s] = jnp.dot(oh, jnp.where(sel, 1.0, 0.0).astype(bf16), preferred_element_type=f32)
        lane, row = _iota((8, 128), 1), _iota((8, 128), 0)
        st['col'] = [(16 * s + lane // 8) % CT == row for s in range(CT)]
        st['acc'] = [jnp.zeros((8, 128), f32)] * 2
        lhs = jnp.concatenate([jnp.where(lane == 8 * (b % 16) + row, oh_s[48 + b // 16:49 + b // 16], 0.0)
                               for b in tail_bands] + [jnp.zeros((8, 128), f32)] * (len(tail_bands) % 2), axis=0)
        hb_s[...] = jnp.dot(lhs.astype(bf16), jnp.ones((128, 128), bf16),
                            preferred_element_type=f32) * ((1.0 - mix_s[1, 0:1]) * mix_s[2, 0:1])

    def out_slice(g):
        def fn():
            mats = ((wo_b, WO_ROWS, 0), (wd_b, WD_ROWS, 48))
            for k, (buf, n, _) in enumerate(mats):
                copy(buf.at[:8 * n], buf.at[:8 * n], S_OUT + 2 * g + k).wait()
            for k, (buf, n, v0) in enumerate(mats):
                for r in range(0 if 'o' in cfg.get('noc', '') else n):
                    blk = r * NG + g
                    a, s = divmod(blk, CT)
                    lhs = jnp.where(st['col'][s], ex_s[s, v0 + a:v0 + a + 1], 0.0).astype(bf16)
                    st['acc'][k] = st['acc'][k] + jnp.dot(lhs, buf[8 * blk:8 * blk + 8].reshape(128, 128),
                                                          preferred_element_type=f32)
        return fn

    first[0][0]().start(priority=0)
    for pc in [pc for pc, queue in first if queue == 1][:LOOK]:
        pc().start(priority=1)
    stream(first[1:], pair_pieces(0), {41: [c.start for c in small_copies], 200: [gates]})

    def pair(p, nxt, before=None, extra=()):
        cur = pair_pieces(p)
        tasks = {}
        spread(tasks, 8, 20, extra)
        if before:
            spread(tasks, LAG, 5, before)
        else:
            spread(tasks, LAG, cfg['step'], pv_slices(p - 1))
        spread(tasks, len(cur) // 2 + LAG, cfg['step'], qk_slices(p))
        assert max(tasks) < len(cur)
        stream(cur, nxt, tasks)

    def body(p, carry):
        pair(p, pair_pieces(p + 1))
        return carry

    pair(0, pair_pieces(1), before=[q_slice(p) for p in range(NP)])
    jax.lax.fori_loop(1, NP - 1, body, 0)
    pair(NP - 1, last, extra=hidden_slices())

    tasks = {}
    spread(tasks, 90, 14, pv_slices(NP - 1, 8) + [expand])
    late = []
    pos = 210
    for g in range(NG):
        pos = max(pos + 14, n_group * (g + 1) + 90)
        if pos < len(last) - LOOK:
            tasks.setdefault(pos, []).append(out_slice(g))
        else:
            late.append(out_slice(g))
    stream(last, [], tasks)
    for fn in late:
        fn()

    x, gate, rsel = mix_s[0], mix_s[1], mix_s[2]
    a, y = st['acc']
    rest = gate * a + (1.0 - gate) * (x + (x * 0.0 + y * rsel))
    acc = [jnp.where(_iota((8, 128), 0) == m, rest, 0.0) for m in range(CT)]
    for sem in sorted({sem for _, _, sem in tail}):
        t0, t1 = min(a for a, _, s in tail if s == sem), max(b for _, b, s in tail if s == sem)
        flat_segment(wd_b, wd_b, sem, t0, t1 - t0)[0]().wait()
        for t in range(t0, t0 if 't' in cfg.get('noc', '') else t1, 2):
            w = wd_b[t // 2].astype(f32)
            for half in range(2):
                band, m = divmod(t + half, CT)
                k = band - tail_bands[0]
                acc[m] = acc[m] + w[8 * half:8 * half + 8] * hb_s[8 * k:8 * k + 8]
    out = jnp.concatenate([jnp.sum(v, axis=0, keepdims=True) for v in acc], axis=1)
    out_ref[0] = out.astype(bf16)


def _memory_order(w):
    r, c = w.shape
    return w.reshape(r // 8, 8, c // 128, 128).transpose(0, 2, 1, 3).reshape(-1, 16, 128)


def make(**kw):
    cfg = dict(look=26, lag=55, step=10, kv=(1, 3), pa=3, pc=4, ns=128, ts=4, tl=2, tg=16)
    cfg.update(kw)

    def fn(A_x, A_k_cache, A_v_cache, A_wq, A_wo, B_x, B_w_r, B_w_gate, B_w_up, B_w_down, gate_w):
        del B_x
        kT = jnp.swapaxes(A_k_cache, 2, 3).reshape(H * DH // 16, 16, SK)
        vT = jnp.swapaxes(A_v_cache, 2, 3).reshape(H * DH // 16, 16, SK)
        wo, wd = _memory_order(A_wo), _memory_order(B_w_down)
        any_spec = pl.BlockSpec(memory_space=pl.ANY)
        vmem = pltpu.VMEM
        return pl.pallas_call(
            functools.partial(_kernel, cfg=cfg),
            out_shape=jax.ShapeDtypeStruct((1, 1, D), bf16),
            in_specs=[any_spec] * 10,
            out_specs=pl.BlockSpec(memory_space=pltpu.VMEM),
            scratch_shapes=[
                vmem((1, 1, D), bf16), vmem((D,), bf16), vmem((D,), bf16),
                vmem((D, H * DH), bf16), vmem((2, PR // 16, 16, W), bf16), vmem((2, PR // 16, 16, W), bf16),
                vmem(wo.shape, bf16), vmem((D, F), bf16), vmem((D, F), bf16), vmem(wd.shape, bf16),
                vmem((NP, 8, PR), f32), vmem((64, 128), f32), vmem((CT, 64, 128), f32),
                vmem((320, 128), f32), vmem((3, 8, 128), f32),
                vmem((8, W), f32), vmem((8, W), f32),
                pltpu.SemaphoreType.DMA((S_TAIL + 48,)),
            ],
            compiler_params=pltpu.CompilerParams(
                vmem_limit_bytes=64 * 1024 * 1024,
                disable_bounds_checks=True,
                disable_semaphore_checks=True,
            ),
            name="gated_mix_decode",
        )(A_x, kT, vT, A_wq, wo, B_w_r, B_w_gate, B_w_up, wd, gate_w)
    return fn


pallas_gated_mix__sliding_block_cached__moe_arch_mod__decode_kernel = jax.jit(make())
```

```python
import functools

import jax
import jax.numpy as jnp
import jax.experimental.pallas as pl
import jax.experimental.pallas.tpu as pltpu

H, DH, SK, D, F = 32, 192, 32768, 640, 1536
W = min(4096, max(256, SK // 4))
NP = H // 2
PR = 2 * DH

LOOK = 26
TILE = 8 * 128
SEG, ROW = 8, 256
SC = 128 * SEG
CT = D // 128
NG = ROW // 16
WO_ROWS, WD_ROWS = H * DH * D // TILE // ROW, F * D // TILE // ROW
TAIL0, TAIL1 = WD_ROWS * ROW, F * D // TILE
TAIL_BANDS = range(TAIL0 // CT, TAIL1 // CT)
O_ROWS = H * DH // 128

S_X, S_WG, S_WU, S_WQ = 0, 3, 4, 5
S_K = S_WQ + H * DH // SC
S_V = S_K + 2 * (W // SC)
S_WO = S_V + 2 * (W // SC)
S_WD = S_WO + NG
S_TAIL = S_WD + NG
N_SEMS = S_TAIL + (TAIL1 - TAIL0) // 16

f32 = jnp.float32
bf16 = jnp.bfloat16


def _iota(shape, dim):
    return jax.lax.broadcasted_iota(jnp.int32, shape, dim)


def _fold(v, rows):
    folded = jnp.zeros((rows, 128), f32)
    for m in range(v.shape[1] // 128):
        folded = jnp.where(_iota((rows, 128), 0) == m, v[0:1, 128 * m:128 * (m + 1)], folded)
    return folded


def _kernel(x_hbm, kT, vT, wq, wo, wr_hbm, wg, wu, wd, gw_hbm, out_ref,
            x_v, wr_v, gw_v, wq_b, k_b, v_b, wo_b, wg_b, wu_b, wd_b,
            q_s, oh_s, ex_s, hb_s, mix_s, s_s, p_s, sems):
    def copy(src, dst, idx, sem):
        return pltpu.make_async_copy(src.at[idx], dst.at[idx], sems.at[sem])

    def wait(buf, idx, sem):
        copy(buf, buf, idx, sem).wait()

    def matrix_segment(src, dst, sem, t):
        nct, pieces, end = src.shape[1] // 128, [], t + SEG
        while t < end:
            band, c = divmod(t, nct)
            n = min(nct - c, end - t)
            pieces.append(functools.partial(copy, src, dst, (pl.ds(8 * band, 8), pl.ds(128 * c, 128 * n)),
                                            sem + (c // SEG if src is wq else 0)))
            t += n
        return pieces

    def wo_piece(r, t):
        return functools.partial(copy, wo, wo_b, (r, pl.ds(t // 2, SEG // 2)), S_WO + t // 16)

    def wd_piece(t, n, sem):
        return functools.partial(copy, wd, wd_b, pl.ds(t // 2, n // 2), sem)

    lead = range(ROW, ROW + ROW // 2, SEG)
    segments = [matrix_segment(wq, wq_b, S_WQ, t) for t in lead]
    segments += [matrix_segment(src, dst, sem, r + t)
                 for parity in range(2) for t in range(0, ROW, SEG)
                 for src, dst, sem in ((wq, wq_b, S_WQ), (wg, wg_b, S_WG), (wu, wu_b, S_WU))
                 for r in range(parity * ROW, src.shape[0] * src.shape[1] // TILE - t, 2 * ROW)
                 if not (src is wq and r + t in lead)]
    first = [(pc, int(i % 3 > 0)) for i, seg in enumerate(segments) for pc in seg]

    def pair_pieces(p):
        def piece(src, buf, sem, r, n, parity, j):
            def make():
                rows = pl.ds(8 * parity, 8)
                return pltpu.make_async_copy(
                    src.at[pl.ds(p * (PR // 16) + r, n), rows, pl.ds(SK - W + j * SC, SC)],
                    buf.at[p % 2, pl.ds(r, n), rows, pl.ds(j * SC, SC)], sems.at[sem + 2 * j + p % 2])
            return make

        blocks = list(range(W // SC))
        return [(piece(src, buf, sem, h + r + queue, (1, 3)[queue], parity, j), queue)
                for src, buf, sem in ((kT, k_b, S_K), (vT, v_b, S_V))
                for h in (0, DH // 16) for parity in range(2) for j in (blocks[::-1] if parity else blocks)
                for r in range(0, DH // 16, 4) for queue in range(2)]

    segments = [pc for t in range(0, ROW, SEG) for parity in range(2)
                for pc in [wo_piece(r, t) for r in range(parity, WO_ROWS, 2)]
                + [wd_piece(r * ROW + t, SEG, S_WD + t // 16) for r in range(parity, WD_ROWS, 2)]]
    last = [(pc, int(i % 4 > 0)) for i, pc in enumerate(segments)]
    solo = TAIL1 - 2 * LOOK
    last += [(wd_piece(t, 4, S_TAIL + (t - TAIL0) // 16), int(t % 32 >= 8)) for t in range(TAIL0, solo, 4)]
    last += [(wd_piece(t, 2, S_TAIL + (t - TAIL0) // 16), 1) for t in range(solo, TAIL1, 2)]

    def stream(cur, nxt, tasks):
        ahead = iter([pc for pc, queue in cur + nxt if queue == 1][LOOK:])
        for i, (pc, queue) in enumerate(cur):
            pc = next(ahead, None) if queue else pc
            if pc is not None:
                pc().start(priority=queue)
            for fn in tasks.get(i, ()):
                fn()

    def spread(start, step, fns):
        return {start + n * step: [fn] for n, fn in enumerate(fns)}

    st = {}
    small = [pltpu.make_async_copy(src, dst, sems.at[S_X + i])
             for i, (src, dst) in enumerate(((x_hbm, x_v), (gw_hbm, gw_v), (wr_hbm, wr_v)))]

    def gates():
        for c in small:
            c.wait()
        x = x_v[0].astype(f32)
        mix_s[0] = _fold(x, 8)
        for i, w in ((1, gw_v), (2, wr_v)):
            z = jnp.sum(x * w[...].astype(f32).reshape(1, D), axis=-1, keepdims=True)
            mix_s[i] = jnp.broadcast_to(jax.nn.sigmoid(z), (8, 128))

    def x_dot(w):
        return jnp.dot(jnp.broadcast_to(x_v[0], (8, D)), w, preferred_element_type=f32)

    def q_proj(j):
        idx = (slice(None), pl.ds(j * SC, SC))
        wait(wq_b, idx, S_WQ + j)
        q = x_dot(wq_b[idx])
        for m in range(SEG):
            q_s[j * SEG + m] = q[:, 128 * m:128 * (m + 1)]

    def gate_proj():
        wait(wg_b, ..., S_WG)
        st['g'] = x_dot(wg_b[...])

    def up_proj():
        wait(wu_b, ..., S_WU)
        oh_s[O_ROWS:] = _fold(jax.nn.silu(st['g']) * x_dot(wu_b[...]), 16)

    def cache_block(buf, sem, p, j):
        idx = (p % 2, slice(None), slice(None), pl.ds(j * SC, SC))
        wait(buf, idx, sem + 2 * j + p % 2)
        return buf[idx].reshape(PR, SC)

    def scores(p, j):
        q = jnp.concatenate([q_s[PR // 128 * p + m] for m in range(PR // 128)], axis=1)
        own = (_iota((8, PR), 1) >= DH) == (_iota((8, PR), 0) % 2 == 1)
        s_s[:, j * SC:(j + 1) * SC] = jnp.dot(jnp.where(own, q, 0.0).astype(bf16), cache_block(k_b, S_K, p, j),
                                              preferred_element_type=f32)

    def softmax():
        sc = s_s[...] * DH ** -0.5
        e = jnp.exp(sc - jnp.max(sc, axis=-1, keepdims=True))
        p_s[...] = e / jnp.sum(e, axis=-1, keepdims=True)

    def attend(p, j):
        o = jax.lax.dot_general(p_s[:, j * SC:(j + 1) * SC].astype(bf16), cache_block(v_b, S_V, p, j),
                                (((1,), (1,)), ((), ())), preferred_element_type=f32)
        st['o'] = o if j == 0 else st['o'] + o
        if j == W // SC - 1:
            o = jnp.where(_iota((1, PR), 1) < DH, st['o'][0:1], st['o'][1:2])
            for m in range(PR // 128):
                oh_s[pl.ds(PR // 128 * p + m, 1)] = o[:, 128 * m:128 * (m + 1)]

    def expand():
        oh = oh_s[...].astype(bf16)
        src, lane = _iota((128, 128), 0), _iota((128, 128), 1)
        for s in range(CT):
            tile = 16 * s + lane // 8 - CT * (src // 8)
            sel = (tile >= 0) & (tile < CT) & (src % 8 == lane % 8)
            ex_s[s] = jnp.dot(oh, jnp.where(sel, 1.0, 0.0).astype(bf16), preferred_element_type=f32)
        lane, row = _iota((8, 128), 1), _iota((8, 128), 0)
        st['col'] = [(16 * s + lane // 8) % CT == row for s in range(CT)]
        st['a'] = st['y'] = jnp.zeros((8, 128), f32)
        picked = [jnp.where(lane == 8 * (b % 16) + row, oh_s[pl.ds(O_ROWS + b // 16, 1)], 0.0) for b in TAIL_BANDS]
        hb = jnp.dot(jnp.concatenate(picked, axis=0).astype(bf16), jnp.ones((128, 128), bf16),
                     preferred_element_type=f32)
        hb_s[...] = hb * ((1.0 - mix_s[1, 0:1]) * mix_s[2, 0:1])

    def block_dot(v0, blk, w):
        a, s = divmod(blk, CT)
        lhs = jnp.where(st['col'][s], ex_s[s, pl.ds(v0 + a, 1)], 0.0).astype(bf16)
        return jnp.dot(lhs, w.reshape(128, 128), preferred_element_type=f32)

    def out_proj(g):
        wait(wo_b, (slice(None), pl.ds(8 * g, 8)), S_WO + g)
        for r in range(WD_ROWS):
            for t in range(16 * g, 16 * (g + 1), SEG):
                wd_piece(r * ROW + t, SEG, S_WD + g)().wait()
        for r in range(WO_ROWS):
            st['a'] = st['a'] + block_dot(0, r * NG + g, wo_b[r, pl.ds(8 * g, 8)])
        for r in range(WD_ROWS):
            st['y'] = st['y'] + block_dot(O_ROWS, r * NG + g, wd_b[pl.ds(8 * (r * NG + g), 8)])

    def each(fn, n, *args):
        return [functools.partial(fn, *args, j) for j in range(n)]

    def pair(p, nxt, tasks):
        cur = pair_pieces(p)
        stream(cur, nxt, tasks | spread(len(cur) // 2 + 55, 10, each(scores, W // SC, p) + [softmax]))

    def middle(p, carry):
        pair(p, pair_pieces(p + 1), spread(55, 16, each(attend, W // SC, p - 1)))
        return carry

    first[0][0]().start(priority=0)
    for pc in [pc for pc, queue in first if queue == 1][:LOOK]:
        pc().start(priority=1)
    stream(first[1:], pair_pieces(0), {41: [c.start for c in small], 200: [gates]})
    pair(0, pair_pieces(1), spread(55, 14, each(q_proj, H * DH // SC)))
    jax.lax.fori_loop(1, NP - 1, middle, 0)
    pair(NP - 1, last, spread(15, 20, [gate_proj, up_proj] + each(attend, W // SC, NP - 2)))

    tasks = spread(90, 26, each(attend, W // SC, NP - 1) + [expand])
    pos = max(tasks)
    for g in range(NG):
        pos = min(max(pos + 14, len(segments) // NG * (g + 1) + 90), len(last) - 1)
        tasks.setdefault(pos, []).append(functools.partial(out_proj, g))
    stream(last, [], tasks)

    x, gate, rsel = mix_s[0], mix_s[1], mix_s[2]
    mixed = gate * st['a'] + (1.0 - gate) * (x + (x * 0.0 + st['y'] * rsel))
    acc = [jnp.where(_iota((8, 128), 0) == m, mixed, 0.0) for m in range(CT)]
    for t in range(TAIL0, TAIL1, 2):
        if t % 16 == 0:
            wait(wd_b, pl.ds(t // 2, 8), S_TAIL + (t - TAIL0) // 16)
        w = wd_b[t // 2].astype(f32)
        for half in range(2):
            band, m = divmod(t + half, CT)
            acc[m] = acc[m] + w[8 * half:8 * half + 8] * hb_s[pl.ds(8 * (band - TAIL_BANDS[0]), 8)]
    out_ref[0] = jnp.concatenate([jnp.sum(v, axis=0, keepdims=True) for v in acc], axis=1).astype(bf16)


def _memory_order(w):
    r, c = w.shape
    return w.reshape(r // 8, 8, c // 128, 128).transpose(0, 2, 1, 3).reshape(-1, 16, 128)


@jax.jit
def pallas_gated_mix__sliding_block_cached__moe_arch_mod__decode_kernel(
        A_x, A_k_cache, A_v_cache, A_wq, A_wo, B_x, B_w_r, B_w_gate, B_w_up, B_w_down, gate_w):
    del B_x
    kT = jnp.swapaxes(A_k_cache, 2, 3).reshape(H * DH // 16, 16, SK)
    vT = jnp.swapaxes(A_v_cache, 2, 3).reshape(H * DH // 16, 16, SK)
    wo = _memory_order(A_wo).reshape(WO_ROWS, ROW // 2, 16, 128)
    wd = _memory_order(B_w_down)
    vmem = pltpu.VMEM
    return pl.pallas_call(
        _kernel,
        out_shape=jax.ShapeDtypeStruct((1, 1, D), bf16),
        in_specs=[pl.BlockSpec(memory_space=pl.ANY)] * 10,
        out_specs=pl.BlockSpec(memory_space=pltpu.VMEM),
        scratch_shapes=[
            vmem((1, 1, D), bf16), vmem((D,), bf16), vmem((D,), bf16),
            vmem((D, H * DH), bf16), vmem((2, PR // 16, 16, W), bf16), vmem((2, PR // 16, 16, W), bf16),
            vmem(wo.shape, bf16), vmem((D, F), bf16), vmem((D, F), bf16), vmem(wd.shape, bf16),
            vmem((O_ROWS, 8, 128), f32), vmem((O_ROWS + 16, 128), f32), vmem((CT, O_ROWS + 16, 128), f32),
            vmem((8 * len(TAIL_BANDS), 128), f32), vmem((3, 8, 128), f32),
            vmem((8, W), f32), vmem((8, W), f32),
            pltpu.SemaphoreType.DMA((N_SEMS,)),
        ],
        compiler_params=pltpu.CompilerParams(
            vmem_limit_bytes=64 * 1024 * 1024,
            disable_semaphore_checks=True,
        ),
        name="gated_mix_decode",
    )(A_x, kT, vT, A_wq, wo, B_w_r, B_w_gate, B_w_up, wd, gate_w)
```

```python
import functools

import jax
import jax.numpy as jnp
import jax.experimental.pallas as pl
import jax.experimental.pallas.tpu as pltpu

H, DH, SK, D, F = 32, 192, 32768, 640, 1536
W = min(4096, max(256, SK // 4))
NP = H // 2
PR = 2 * DH

PB = PR // 8
UNIT = 32
RING = 4
LOOK = 26
TILE = 8 * 128
SEG, ROW = 8, 256
SC = 128 * SEG
CT = D // 128
NG = ROW // 16
WO_ROWS, WD_ROWS = H * DH * D // TILE // ROW, F * D // TILE // ROW
TAIL0, TAIL1 = WD_ROWS * ROW, F * D // TILE
TAIL_BANDS = range(TAIL0 // CT, TAIL1 // CT)
O_ROWS = H * DH // 128

S_X, S_WG, S_WU, S_WQ = 0, 3, 4, 5
S_K = S_WQ + H * DH // SC
S_V = S_K + (RING + 1) * (W // SC)
S_WO = S_V + (RING + 1) * (W // SC)
S_WD = S_WO + NG
S_TAIL = S_WD + NG
N_SEMS = S_TAIL + (TAIL1 - TAIL0) // 8

f32 = jnp.float32
bf16 = jnp.bfloat16


def _iota(shape, dim):
    return jax.lax.broadcasted_iota(jnp.int32, shape, dim)


def _fold(v, rows):
    folded = jnp.zeros((rows, 128), f32)
    for m in range(v.shape[1] // 128):
        folded = jnp.where(_iota((rows, 128), 0) == m, v[0:1, 128 * m:128 * (m + 1)], folded)
    return folded


def _kernel(x_hbm, kT, vT, wq, wo, wr_hbm, wg, wu, wd, gw_hbm, out_ref,
            x_v, wr_v, gw_v, wq_b, k_b, v_b, wo_b, wg_b, wu_b, wd_b,
            q_s, oh_s, ex_s, hb_s, mix_s, s_s, p_s, t_s, sems, *, cfg):
    def copy(src, dst, idx, sem):
        return pltpu.make_async_copy(src.at[idx], dst.at[idx], sems.at[sem])

    def wait(buf, idx, sem):
        copy(buf, buf, idx, sem).wait()

    def matrix_segment(src, dst, sem, t):
        nct, pieces, end = src.shape[1] // 128, [], t + SEG
        while t < end:
            band, c = divmod(t, nct)
            n = min(nct - c, end - t)
            pieces.append(functools.partial(copy, src, dst, (pl.ds(8 * band, 8), pl.ds(128 * c, 128 * n)),
                                            sem + (c // SEG if src is wq else 0)))
            t += n
        return pieces

    def wo_piece(r, t):
        return functools.partial(copy, wo, wo_b, (r, pl.ds(t // 2, SEG // 2)), S_WO + t // 16)

    def wd_piece(t, n, sem):
        return functools.partial(copy, wd, wd_b, pl.ds(t // 2, n // 2), sem)

    lead = range(ROW, ROW + cfg['ns'], SEG)
    segments = [matrix_segment(wq, wq_b, S_WQ, t) for t in lead]
    segments += [matrix_segment(src, dst, sem, r + t)
                 for parity in range(2) for t in range(0, ROW, SEG)
                 for src, dst, sem in ((wq, wq_b, S_WQ), (wg, wg_b, S_WG), (wu, wu_b, S_WU))
                 for r in range(parity * ROW, src.shape[0] * src.shape[1] // TILE - t, 2 * ROW)
                 if not (src is wq and r + t in lead)]
    first = [(pc, int(i % cfg['pa'] > 0)) for i, seg in enumerate(segments) for pc in seg]

    def slot(p):
        if isinstance(p, int):
            return RING if p % NP == NP - 1 else p % RING
        return jnp.where(p % NP == NP - 1, RING, p % RING)

    SH, PERM = cfg['sh'], cfg['perm']

    def cache_pieces(u):
        def piece(src, buf, sem, row, to, off, j):
            return lambda: pltpu.make_async_copy(src.at[pl.ds(row, 8), pl.ds(SK - W + j * SC, SC)],
                                                 buf.at[to, pl.ds(off, 8), pl.ds(j * SC, SC)],
                                                 sems.at[sem + (RING + 1) * j + to])

        pieces, blocks = [], list(range(W // SC))
        for src, buf, sem, shift, order in zip((kT, vT), (k_b, v_b), (S_K, S_V), SH, PERM):
            p, b0 = divmod(UNIT * u - shift + NP * PB, PB)
            here, there = (PR * (p % NP), slot(p)), (PR * ((p + 1) % NP), slot(p + 1))
            bands = []
            for b in order:
                over = b0 + b >= PB
                if isinstance(u, int):
                    (base, to), off = there if over else here, 8 * ((b0 + b) % PB)
                    bands.append((base + off, to, off))
                else:
                    base, to = (jnp.where(over, y, x) for x, y in zip(here, there))
                    off = 8 * jnp.where(over, b0 + b - PB, b0 + b)
                    bands.append((pl.multiple_of(base + off, 8), to, pl.multiple_of(off, 8)))
            for half in range(2):
                pieces += [piece(src, buf, sem, *band, j) for j in (blocks[::-1] if half else blocks)
                           for band in bands[UNIT // 2 * half:UNIT // 2 * (half + 1)]]
        return [(pc, int(n % 4 > 0)) for n, pc in enumerate(pieces)]

    segments = [pc for t in range(0, ROW, SEG) for parity in range(2)
                for pc in [wo_piece(r, t) for r in range(parity, WO_ROWS, 2)]
                + [wd_piece(r * ROW + t, SEG, S_WD + t // 16) for r in range(parity, WD_ROWS, 2)]]
    last = [(pc, int(i % cfg['pc'] > 0)) for i, pc in enumerate(segments)]
    TG = cfg['tg']
    solo = TAIL1 - 2 * LOOK
    last += [(wd_piece(t, 4, S_TAIL + (t - TAIL0) // TG), int(t % cfg['tp'] >= 8)) for t in range(TAIL0, solo, 4)]
    last += [(wd_piece(t, 2, S_TAIL + (t - TAIL0) // TG), 1) for t in range(solo, TAIL1, 2)]

    def stream(cur, nxt, tasks):
        ahead = iter([pc for pc, queue in cur + nxt if queue == 1][LOOK:])
        for i, (pc, queue) in enumerate(cur):
            pc = next(ahead, None) if queue else pc
            if pc is not None:
                pc().start(priority=queue)
            for fn in tasks.get(i, ()):
                fn()

    def spread(start, step, fns):
        return {start + n * step: [fn] for n, fn in enumerate(fns)}

    st = {}
    small = [pltpu.make_async_copy(src, dst, sems.at[S_X + i])
             for i, (src, dst) in enumerate(((x_hbm, x_v), (gw_hbm, gw_v), (wr_hbm, wr_v)))]

    def gates():
        for c in small:
            c.wait()
        x = x_v[0].astype(f32)
        mix_s[0] = _fold(x, 8)
        for i, w in ((1, gw_v), (2, wr_v)):
            z = jnp.sum(x * w[...].astype(f32).reshape(1, D), axis=-1, keepdims=True)
            mix_s[i] = jnp.broadcast_to(jax.nn.sigmoid(z), (8, 128))

    def x_dot(w):
        return jnp.dot(jnp.broadcast_to(x_v[0], (8, D)), w, preferred_element_type=f32)

    def q_proj(j):
        idx = (slice(None), pl.ds(j * SC, SC))
        wait(wq_b, idx, S_WQ + j)
        q = x_dot(wq_b[idx])
        for m in range(SEG):
            q_s[j * SEG + m] = q[:, 128 * m:128 * (m + 1)]

    def gate_proj():
        wait(wg_b, ..., S_WG)
        t_s[...] = x_dot(wg_b[...])

    def up_proj():
        wait(wu_b, ..., S_WU)
        oh_s[O_ROWS:] = _fold(jax.nn.silu(t_s[...]) * x_dot(wu_b[...]), 16)

    def cache_block(buf, sem, p, j):
        idx = (slot(p), slice(None), pl.ds(j * SC, SC))
        wait(buf, idx, sem + (RING + 1) * j + slot(p))
        return buf[idx]

    def scores(p, j):
        q = jnp.concatenate([q_s[PR // 128 * p + m] for m in range(PR // 128)], axis=1)
        own = (_iota((8, PR), 1) >= DH) == (_iota((8, PR), 0) % 2 == 1)
        s_s[:, j * SC:(j + 1) * SC] = jnp.dot(jnp.where(own, q, 0.0).astype(bf16), cache_block(k_b, S_K, p, j),
                                              preferred_element_type=f32)

    def softmax():
        sc = s_s[...] * DH ** -0.5
        e = jnp.exp(sc - jnp.max(sc, axis=-1, keepdims=True))
        p_s[...] = e / jnp.sum(e, axis=-1, keepdims=True)

    def attend(p, j):
        o = jax.lax.dot_general(p_s[:, j * SC:(j + 1) * SC].astype(bf16), cache_block(v_b, S_V, p, j),
                                (((1,), (1,)), ((), ())), preferred_element_type=f32)
        o = o if j == 0 else t_s[:, :PR] + o
        if j < W // SC - 1:
            t_s[:, :PR] = o
        else:
            o = jnp.where(_iota((1, PR), 1) < DH, o[0:1], o[1:2])
            for m in range(PR // 128):
                oh_s[pl.ds(PR // 128 * p + m, 1)] = o[:, 128 * m:128 * (m + 1)]

    def expand():
        oh = oh_s[...].astype(bf16)
        src, lane = _iota((128, 128), 0), _iota((128, 128), 1)
        for s in range(CT):
            tile = 16 * s + lane // 8 - CT * (src // 8)
            sel = (tile >= 0) & (tile < CT) & (src % 8 == lane % 8)
            ex_s[s] = jnp.dot(oh, jnp.where(sel, 1.0, 0.0).astype(bf16), preferred_element_type=f32)
        lane, row = _iota((8, 128), 1), _iota((8, 128), 0)
        st['col'] = [(16 * s + lane // 8) % CT == row for s in range(CT)]
        st['a'] = st['y'] = jnp.zeros((8, 128), f32)
        picked = [jnp.where(lane == 8 * (b % 16) + row, oh_s[pl.ds(O_ROWS + b // 16, 1)], 0.0) for b in TAIL_BANDS]
        hb = jnp.dot(jnp.concatenate(picked, axis=0).astype(bf16), jnp.ones((128, 128), bf16),
                     preferred_element_type=f32)
        hb_s[...] = hb * ((1.0 - mix_s[1, 0:1]) * mix_s[2, 0:1])

    def block_dot(v0, blk, w):
        a, s = divmod(blk, CT)
        lhs = jnp.where(st['col'][s], ex_s[s, pl.ds(v0 + a, 1)], 0.0).astype(bf16)
        return jnp.dot(lhs, w.reshape(128, 128), preferred_element_type=f32)

    def out_proj(g):
        wait(wo_b, (slice(None), pl.ds(8 * g, 8)), S_WO + g)
        for r in range(WD_ROWS):
            for t in range(16 * g, 16 * (g + 1), SEG):
                wd_piece(r * ROW + t, SEG, S_WD + g)().wait()
        for r in range(WO_ROWS):
            st['a'] = st['a'] + block_dot(0, r * NG + g, wo_b[r, pl.ds(8 * g, 8)])
        for r in range(WD_ROWS):
            st['y'] = st['y'] + block_dot(O_ROWS, r * NG + g, wd_b[pl.ds(8 * (r * NG + g), 8)])

    def each(fn, n, *args):
        return [functools.partial(fn, *args, j) for j in range(n)]

    def attention(p):
        return each(scores, W // SC, p) + [softmax] + each(attend, W // SC, p)

    def step(u, carry):
        p, b0 = divmod(UNIT * u - max(SH) + PB, PB)
        tasks = spread(20, 24, [functools.partial(pl.when((b0 < UNIT) & (p >= 2)), fn) for fn in attention(p - 2)])
        tasks |= spread(21, 27, [functools.partial(pl.when(u == 1), fn)
                                 for fn in each(q_proj, H * DH // SC) + [gate_proj, up_proj]])
        cur = cache_pieces(u)
        stream(cur[:-40], cur[-40:], tasks)
        pl.when(u < n_steps - 1)(lambda: stream(cur[-40:], cache_pieces(u + 1), {}))
        return carry

    n_steps = NP * PB // UNIT
    first[0][0]().start(priority=0)
    for pc in [pc for pc, queue in first if queue == 1][:LOOK]:
        pc().start(priority=1)
    stream(first[1:], cache_pieces(0), {41: [c.start for c in small], 200: [gates]})
    jax.lax.fori_loop(0, n_steps, step, 0)
    stream(cache_pieces(n_steps - 1)[-40:], last, {})

    done = (UNIT * (n_steps - 1) - max(SH)) // PB
    tasks = spread(10, cfg['t1'], [fn for p in range(done, NP) for fn in attention(p)] + [expand])
    pos = max(tasks)
    for g in range(NG):
        pos = min(max(pos + 12, len(segments) // NG * (g + 1) + 90), len(last) - 1)
        tasks.setdefault(pos, []).append(functools.partial(out_proj, g))
    stream(last, [], tasks)

    x, gate, rsel = mix_s[0], mix_s[1], mix_s[2]
    mixed = gate * st['a'] + (1.0 - gate) * (x + (x * 0.0 + st['y'] * rsel))
    acc = [jnp.where(_iota((8, 128), 0) == m, mixed, 0.0) for m in range(CT)]
    for t in range(TAIL0, TAIL1, 2):
        if t % TG == 0:
            wait(wd_b, pl.ds(t // 2, TG // 2), S_TAIL + (t - TAIL0) // TG)
        w = wd_b[t // 2].astype(f32)
        for half in range(2):
            band, m = divmod(t + half, CT)
            acc[m] = acc[m] + w[8 * half:8 * half + 8] * hb_s[pl.ds(8 * (band - TAIL_BANDS[0]), 8)]
    out_ref[0] = jnp.concatenate([jnp.sum(v, axis=0, keepdims=True) for v in acc], axis=1).astype(bf16)


def _memory_order(w):
    r, c = w.shape
    return w.reshape(r // 8, 8, c // 128, 128).transpose(0, 2, 1, 3).reshape(-1, 16, 128)


def make(**kw):
    cfg = dict(pa=3, pc=4, ns=128, tg=16, tp=32, nobounds=True, sh=(27, 18), t1=18, perm=(tuple(range(0, 32, 2)) + tuple(range(1, 32, 2)),) * 2)
    cfg.update(kw)

    def fn(A_x, A_k_cache, A_v_cache, A_wq, A_wo, B_x, B_w_r, B_w_gate, B_w_up, B_w_down, gate_w):
        del B_x
        kT = jnp.swapaxes(A_k_cache, 2, 3).reshape(H * DH, SK)
        vT = jnp.swapaxes(A_v_cache, 2, 3).reshape(H * DH, SK)
        wo = _memory_order(A_wo).reshape(WO_ROWS, ROW // 2, 16, 128)
        wd = _memory_order(B_w_down)
        vmem = pltpu.VMEM
        return pl.pallas_call(
            functools.partial(_kernel, cfg=cfg),
            out_shape=jax.ShapeDtypeStruct((1, 1, D), bf16),
            in_specs=[pl.BlockSpec(memory_space=pl.ANY)] * 10,
            out_specs=pl.BlockSpec(memory_space=pltpu.VMEM),
            scratch_shapes=[
                vmem((1, 1, D), bf16), vmem((D,), bf16), vmem((D,), bf16),
                vmem((D, H * DH), bf16), vmem((RING + 1, PR, W), bf16), vmem((RING + 1, PR, W), bf16),
                vmem(wo.shape, bf16), vmem((D, F), bf16), vmem((D, F), bf16), vmem(wd.shape, bf16),
                vmem((O_ROWS, 8, 128), f32), vmem((O_ROWS + 16, 128), f32), vmem((CT, O_ROWS + 16, 128), f32),
                vmem((8 * len(TAIL_BANDS), 128), f32), vmem((3, 8, 128), f32),
                vmem((8, W), f32), vmem((8, W), f32), vmem((8, F), f32),
                pltpu.SemaphoreType.DMA((N_SEMS,)),
            ],
            compiler_params=pltpu.CompilerParams(
                vmem_limit_bytes=80 * 1024 * 1024,
                disable_bounds_checks=cfg['nobounds'],
                disable_semaphore_checks=True,
            ),
            name="gated_mix_decode",
        )(A_x, kT, vT, A_wq, wo, B_w_r, B_w_gate, B_w_up, wd, gate_w)
    return fn


pallas_gated_mix__sliding_block_cached__moe_arch_mod__decode_kernel = jax.jit(make())
```

```python
import functools

import jax
import jax.numpy as jnp
import jax.experimental.pallas as pl
import jax.experimental.pallas.tpu as pltpu

H, DH, SK, D, F = 32, 192, 32768, 640, 1536
W = min(4096, max(256, SK // 4))
NP = H // 2
PR = 2 * DH
PB = PR // 8
RING = 4
UNIT = 32

LOOK = 26
TILE = 8 * 128
SEG, ROW = 8, 256
SC = 128 * SEG
CT = D // 128
NG = ROW // 16
WO_ROWS, WD_ROWS = H * DH * D // TILE // ROW, F * D // TILE // ROW
TAIL0, TAIL1 = WD_ROWS * ROW, F * D // TILE
TAIL_BANDS = range(TAIL0 // CT, TAIL1 // CT)
O_ROWS = H * DH // 128

K_SHIFT, V_SHIFT = 27, 18
WG_TURN, WU_TURN, WD_TURN = (9, 10), (1, 2), (12, 13)

S_X, S_WG, S_WU, S_WQ = 0, 3, 4, 5
S_K = S_WQ + H * DH // SC
S_V = S_K + (RING + 1) * (W // SC)
S_WO = S_V + (RING + 1) * (W // SC)
S_WD = S_WO + NG
S_TAIL = S_WD + NG
N_SEMS = S_TAIL + (TAIL1 - TAIL0) // 16

f32 = jnp.float32
bf16 = jnp.bfloat16


def _iota(shape, dim):
    return jax.lax.broadcasted_iota(jnp.int32, shape, dim)


def _select(cond, a, b):
    return (a if cond else b) if isinstance(cond, bool) else jnp.where(cond, a, b)


def _band(row):
    return pl.ds(row if isinstance(row, int) else pl.multiple_of(row, 8), 8)


def _slot(p):
    return _select(p % NP == NP - 1, RING, p % RING)


def _fold(v, rows):
    folded = jnp.zeros((rows, 128), f32)
    for m in range(v.shape[1] // 128):
        folded = jnp.where(_iota((rows, 128), 0) == m, v[0:1, 128 * m:128 * (m + 1)], folded)
    return folded


def _kernel(x_hbm, kT, vT, wq, wo, wr_hbm, wg, wu, wd, gw_hbm, out_ref,
            x_v, wr_v, gw_v, wq_b, k_b, v_b, wo_b, wg_b, wu_b, wd_b,
            q_s, oh_s, ex_s, hb_s, mix_s, s_s, p_s, t_s, sems):
    def copy(src, dst, idx, sem):
        return pltpu.make_async_copy(src.at[idx], dst.at[idx], sems.at[sem])

    def wait(buf, idx, sem):
        copy(buf, buf, idx, sem).wait()

    def matrix_segment(src, dst, sem, t):
        nct, pieces, end = src.shape[1] // 128, [], t + SEG
        while t < end:
            band, c = divmod(t, nct)
            n = min(nct - c, end - t)
            pieces.append(functools.partial(copy, src, dst, (_band(8 * band), pl.ds(128 * c, 128 * n)),
                                            sem + (c // SEG if src is wq else 0)))
            t += n
        return pieces

    lead = range(ROW, ROW + ROW // 2, SEG)
    segments = [matrix_segment(wq, wq_b, S_WQ, t) for t in lead]
    for parity in range(2):
        for t in range(0, ROW, SEG):
            for src, dst, sem, turn in ((wq, wq_b, S_WQ, 0), (wg, wg_b, S_WG, WG_TURN[parity]),
                                        (wu, wu_b, S_WU, WU_TURN[parity])):
                size = src.shape[0] * src.shape[1] // TILE
                segments += [matrix_segment(src, dst, sem, r + (t + SEG * turn) % min(ROW, size - r))
                             for r in range(parity * ROW, size - t, 2 * ROW)
                             if not (src is wq and r + t in lead)]
    first = [(pc, int(i % 3 > 0)) for i, seg in enumerate(segments) for pc in seg]

    def cache_pieces(u):
        def piece(src, buf, sem, rows, slot, slot_rows, j):
            return lambda: pltpu.make_async_copy(src.at[rows, pl.ds(SK - W + j * SC, SC)],
                                                 buf.at[slot, slot_rows, pl.ds(j * SC, SC)],
                                                 sems.at[sem + (RING + 1) * j + slot])

        pieces, blocks = [], list(range(W // SC))
        for src, buf, sem, shift in ((kT, k_b, S_K, K_SHIFT), (vT, v_b, S_V, V_SHIFT)):
            p, b0 = divmod(UNIT * u - shift + NP * PB, PB)
            here, there = (PR * (p % NP), _slot(p)), (PR * ((p + 1) % NP), _slot(p + 1))
            bands = []
            for b in range(UNIT):
                over = b0 + b >= PB
                base, slot = (_select(over, y, x) for x, y in zip(here, there))
                off = 8 * _select(over, b0 + b - PB, b0 + b)
                bands.append((_band(base + off), slot, _band(off)))
            pieces += [piece(src, buf, sem, *band, j) for parity in range(2)
                       for j in (blocks[::-1] if parity else blocks) for band in bands[parity::2]]
        return [(pc, int(i % 4 > 0)) for i, pc in enumerate(pieces)]

    def wo_piece(r, t):
        return functools.partial(copy, wo, wo_b, (r, pl.ds(t // 2, SEG // 2)), S_WO + t // 16)

    def wd_piece(t, n, sem):
        return functools.partial(copy, wd, wd_b, pl.ds(t // 2, n // 2), sem)

    swept = [pc for t in range(0, ROW, SEG) for parity in range(2)
             for pc in [wo_piece(r, t) for r in range(parity, WO_ROWS, 2)]
             + [wd_piece(r * ROW + (t + 16 * WD_TURN[parity]) % ROW, SEG, S_WD + t // 16)
                for r in range(parity, WD_ROWS, 2)]]
    last = [(pc, int(i % 4 > 0)) for i, pc in enumerate(swept)]
    solo = TAIL1 - 2 * LOOK
    last += [(wd_piece(t, 4, S_TAIL + (t - TAIL0) // 16), int(t % 32 >= 8)) for t in range(TAIL0, solo, 4)]
    last += [(wd_piece(t, 2, S_TAIL + (t - TAIL0) // 16), 1) for t in range(solo, TAIL1, 2)]

    def stream(cur, nxt, tasks):
        ahead = iter([pc for pc, queue in cur + nxt if queue == 1][LOOK:])
        for i, (pc, queue) in enumerate(cur):
            pc = next(ahead, None) if queue else pc
            if pc is not None:
                pc().start(priority=queue)
            for fn in tasks.get(i, ()):
                fn()

    st = {}
    small = [pltpu.make_async_copy(src, dst, sems.at[S_X + i])
             for i, (src, dst) in enumerate(((x_hbm, x_v), (gw_hbm, gw_v), (wr_hbm, wr_v)))]

    def gates():
        for c in small:
            c.wait()
        x = x_v[0].astype(f32)
        mix_s[0] = _fold(x, 8)
        for i, w in ((1, gw_v), (2, wr_v)):
            z = jnp.sum(x * w[...].astype(f32).reshape(1, D), axis=-1, keepdims=True)
            mix_s[i] = jnp.broadcast_to(jax.nn.sigmoid(z), (8, 128))

    def x_dot(w):
        return jnp.dot(jnp.broadcast_to(x_v[0], (8, D)), w, preferred_element_type=f32)

    def q_proj(j):
        idx = (slice(None), pl.ds(j * SC, SC))
        wait(wq_b, idx, S_WQ + j)
        q = x_dot(wq_b[idx])
        for m in range(SEG):
            q_s[j * SEG + m] = q[:, 128 * m:128 * (m + 1)]

    def gate_proj():
        wait(wg_b, ..., S_WG)
        t_s[...] = x_dot(wg_b[...])

    def up_proj():
        wait(wu_b, ..., S_WU)
        oh_s[O_ROWS:] = _fold(jax.nn.silu(t_s[...]) * x_dot(wu_b[...]), 16)

    def cache_block(buf, sem, p, j):
        idx = (_slot(p), slice(None), pl.ds(j * SC, SC))
        wait(buf, idx, sem + (RING + 1) * j + _slot(p))
        return buf[idx]

    def scores(p, j):
        q = jnp.concatenate([q_s[PR // 128 * p + m] for m in range(PR // 128)], axis=1)
        own = (_iota((8, PR), 1) >= DH) == (_iota((8, PR), 0) % 2 == 1)
        s_s[:, j * SC:(j + 1) * SC] = jnp.dot(jnp.where(own, q, 0.0).astype(bf16), cache_block(k_b, S_K, p, j),
                                              preferred_element_type=f32)

    def softmax():
        sc = s_s[...] * DH ** -0.5
        e = jnp.exp(sc - jnp.max(sc, axis=-1, keepdims=True))
        p_s[...] = e / jnp.sum(e, axis=-1, keepdims=True)

    def attend(p, j):
        o = jax.lax.dot_general(p_s[:, j * SC:(j + 1) * SC].astype(bf16), cache_block(v_b, S_V, p, j),
                                (((1,), (1,)), ((), ())), preferred_element_type=f32)
        o = o if j == 0 else t_s[:, :PR] + o
        if j < W // SC - 1:
            t_s[:, :PR] = o
        else:
            o = jnp.where(_iota((1, PR), 1) < DH, o[0:1], o[1:2])
            for m in range(PR // 128):
                oh_s[pl.ds(PR // 128 * p + m, 1)] = o[:, 128 * m:128 * (m + 1)]

    def expand():
        oh = oh_s[...].astype(bf16)
        src, lane = _iota((128, 128), 0), _iota((128, 128), 1)
        for s in range(CT):
            tile = 16 * s + lane // 8 - CT * (src // 8)
            sel = (tile >= 0) & (tile < CT) & (src % 8 == lane % 8)
            ex_s[s] = jnp.dot(oh, jnp.where(sel, 1.0, 0.0).astype(bf16), preferred_element_type=f32)
        lane, row = _iota((8, 128), 1), _iota((8, 128), 0)
        st['col'] = [(16 * s + lane // 8) % CT == row for s in range(CT)]
        st['a'] = st['y'] = jnp.zeros((8, 128), f32)
        picked = [jnp.where(lane == 8 * (b % 16) + row, oh_s[pl.ds(O_ROWS + b // 16, 1)], 0.0) for b in TAIL_BANDS]
        hb = jnp.dot(jnp.concatenate(picked, axis=0).astype(bf16), jnp.ones((128, 128), bf16),
                     preferred_element_type=f32)
        hb_s[...] = hb * ((1.0 - mix_s[1, 0:1]) * mix_s[2, 0:1])

    def block_dot(v0, blk, w):
        a, s = divmod(blk, CT)
        lhs = jnp.where(st['col'][s], ex_s[s, pl.ds(v0 + a, 1)], 0.0).astype(bf16)
        return jnp.dot(lhs, w.reshape(128, 128), preferred_element_type=f32)

    def out_proj(g):
        wait(wo_b, (slice(None), pl.ds(8 * g, 8)), S_WO + g)
        down = [r * NG + (g + WD_TURN[r % 2]) % NG for r in range(WD_ROWS)]
        for blk in down:
            for t in range(16 * blk, 16 * (blk + 1), SEG):
                wd_piece(t, SEG, S_WD + g)().wait()
        for r in range(WO_ROWS):
            st['a'] = st['a'] + block_dot(0, r * NG + g, wo_b[r, pl.ds(8 * g, 8)])
        for blk in down:
            st['y'] = st['y'] + block_dot(O_ROWS, blk, wd_b[pl.ds(8 * blk, 8)])

    def spread(start, step, fns):
        return {start + n * step: [fn] for n, fn in enumerate(fns)}

    def each(fn, n, *args):
        return [functools.partial(fn, *args, j) for j in range(n)]

    def attention(p):
        return each(scores, W // SC, p) + [softmax] + each(attend, W // SC, p)

    n_steps, shift = NP * PB // UNIT, max(K_SHIFT, V_SHIFT)

    def step(u, carry):
        p, b0 = divmod(UNIT * u - shift + PB, PB)
        tasks = spread(20, 24, [functools.partial(pl.when((b0 < UNIT) & (p >= 2)), fn) for fn in attention(p - 2)])
        tasks |= spread(21, 27, [functools.partial(pl.when(u == 1), fn)
                                 for fn in each(q_proj, H * DH // SC) + [gate_proj, up_proj]])
        cur = cache_pieces(u)
        stream(cur[:-40], cur[-40:], tasks)
        pl.when(u < n_steps - 1)(lambda: stream(cur[-40:], cache_pieces(u + 1), {}))
        return carry

    first[0][0]().start(priority=0)
    for pc in [pc for pc, queue in first if queue == 1][:LOOK]:
        pc().start(priority=1)
    stream(first[1:], cache_pieces(0), {41: [c.start for c in small], 200: [gates]})
    jax.lax.fori_loop(0, n_steps, step, 0)
    stream(cache_pieces(n_steps - 1)[-40:], last, {})

    done = (UNIT * (n_steps - 1) - shift) // PB
    tasks = spread(10, 18, [fn for p in range(done, NP) for fn in attention(p)] + [expand])
    pos = max(tasks)
    for g in range(NG):
        pos = min(max(pos + 12, len(swept) // NG * (g + 1) + 90), len(last) - 1)
        tasks.setdefault(pos, []).append(functools.partial(out_proj, g))
    stream(last, [], tasks)

    x, gate, rsel = mix_s[0], mix_s[1], mix_s[2]
    mixed = gate * st['a'] + (1.0 - gate) * (x + (x * 0.0 + st['y'] * rsel))
    acc = [jnp.where(_iota((8, 128), 0) == m, mixed, 0.0) for m in range(CT)]
    for t in range(TAIL0, TAIL1, 2):
        if t % 16 == 0:
            wait(wd_b, pl.ds(t // 2, 8), S_TAIL + (t - TAIL0) // 16)
        w = wd_b[t // 2].astype(f32)
        for half in range(2):
            band, m = divmod(t + half, CT)
            acc[m] = acc[m] + w[8 * half:8 * half + 8] * hb_s[pl.ds(8 * (band - TAIL_BANDS[0]), 8)]
    out_ref[0] = jnp.concatenate([jnp.sum(v, axis=0, keepdims=True) for v in acc], axis=1).astype(bf16)


def _memory_order(w):
    r, c = w.shape
    return w.reshape(r // 8, 8, c // 128, 128).transpose(0, 2, 1, 3).reshape(-1, 16, 128)


@jax.jit
def pallas_gated_mix__sliding_block_cached__moe_arch_mod__decode_kernel(
        A_x, A_k_cache, A_v_cache, A_wq, A_wo, B_x, B_w_r, B_w_gate, B_w_up, B_w_down, gate_w):
    del B_x
    kT = jnp.swapaxes(A_k_cache, 2, 3).reshape(H * DH, SK)
    vT = jnp.swapaxes(A_v_cache, 2, 3).reshape(H * DH, SK)
    wo = _memory_order(A_wo).reshape(WO_ROWS, ROW // 2, 16, 128)
    wd = _memory_order(B_w_down)
    vmem = pltpu.VMEM
    return pl.pallas_call(
        _kernel,
        out_shape=jax.ShapeDtypeStruct((1, 1, D), bf16),
        in_specs=[pl.BlockSpec(memory_space=pl.ANY)] * 10,
        out_specs=pl.BlockSpec(memory_space=pltpu.VMEM),
        scratch_shapes=[
            vmem((1, 1, D), bf16), vmem((D,), bf16), vmem((D,), bf16),
            vmem((D, H * DH), bf16), vmem((RING + 1, PR, W), bf16), vmem((RING + 1, PR, W), bf16),
            vmem(wo.shape, bf16), vmem((D, F), bf16), vmem((D, F), bf16), vmem(wd.shape, bf16),
            vmem((O_ROWS, 8, 128), f32), vmem((O_ROWS + 16, 128), f32), vmem((CT, O_ROWS + 16, 128), f32),
            vmem((8 * len(TAIL_BANDS), 128), f32), vmem((3, 8, 128), f32),
            vmem((8, W), f32), vmem((8, W), f32), vmem((8, F), f32),
            pltpu.SemaphoreType.DMA((N_SEMS,)),
        ],
        compiler_params=pltpu.CompilerParams(
            vmem_limit_bytes=80 * 1024 * 1024,
            disable_bounds_checks=True,
            disable_semaphore_checks=True,
        ),
        name="gated_mix_decode",
    )(A_x, kT, vT, A_wq, wo, B_w_r, B_w_gate, B_w_up, wd, gate_w)
```

```python
import functools

import jax
import jax.numpy as jnp
import jax.experimental.pallas as pl
import jax.experimental.pallas.tpu as pltpu

H, DH, SK, D, F = 32, 192, 32768, 640, 1536
W = min(4096, max(256, SK // 4))
NP = H // 2
PR = 2 * DH
PB = PR // 8
RING = 4
UNIT = 32

LOOK = 26
TILE = 8 * 128
SEG, ROW = 8, 256
SC = 128 * SEG
CT = D // 128
NG = ROW // 16
WO_ROWS, WD_ROWS = H * DH * D // TILE // ROW, F * D // TILE // ROW
TAIL0, TAIL1 = WD_ROWS * ROW, F * D // TILE
TAIL_BANDS = range(TAIL0 // CT, TAIL1 // CT)
O_ROWS = H * DH // 128

K_SHIFT, V_SHIFT = 27, 18
K_ORDER = (24, 30, 8, 14, 10, 26, 12, 28, 6, 4, 2, 0, 16, 22, 20, 18,
           9, 13, 29, 31, 25, 15, 19, 3, 21, 17, 23, 27, 1, 5, 7, 11)
V_ORDER = (26, 28, 24, 8, 12, 10, 30, 14, 22, 16, 0, 6, 4, 2, 18, 20,
           5, 19, 3, 1, 7, 17, 11, 9, 23, 15, 13, 21, 29, 25, 27, 31)
WO_ORDER = (9, 5, 7, 3, 1, 8, 11, 13), (0, 2, 6, 10, 4, 12, 14)
WG_TURN, WU_TURN, WD_TURN = (9, 10), (1, 2), (12, 13)

S_X, S_WG, S_WU, S_WQ = 0, 3, 4, 5
S_K = S_WQ + H * DH // SC
S_V = S_K + (RING + 1) * (W // SC)
S_WO = S_V + (RING + 1) * (W // SC)
S_WD = S_WO + NG
S_TAIL = S_WD + NG
N_SEMS = S_TAIL + (TAIL1 - TAIL0) // 16

f32 = jnp.float32
bf16 = jnp.bfloat16


def _iota(shape, dim):
    return jax.lax.broadcasted_iota(jnp.int32, shape, dim)


def _select(cond, a, b):
    return (a if cond else b) if isinstance(cond, bool) else jnp.where(cond, a, b)


def _band(row):
    return pl.ds(row if isinstance(row, int) else pl.multiple_of(row, 8), 8)


def _slot(p):
    return _select(p % NP == NP - 1, RING, p % RING)


def _fold(v, rows):
    folded = jnp.zeros((rows, 128), f32)
    for m in range(v.shape[1] // 128):
        folded = jnp.where(_iota((rows, 128), 0) == m, v[0:1, 128 * m:128 * (m + 1)], folded)
    return folded


def _kernel(x_hbm, kT, vT, wq, wo, wr_hbm, wg, wu, wd, gw_hbm, out_ref,
            x_v, wr_v, gw_v, wq_b, k_b, v_b, wo_b, wg_b, wu_b, wd_b,
            q_s, oh_s, ex_s, hb_s, mix_s, s_s, p_s, t_s, sems):
    def copy(src, dst, idx, sem):
        return pltpu.make_async_copy(src.at[idx], dst.at[idx], sems.at[sem])

    def wait(buf, idx, sem):
        copy(buf, buf, idx, sem).wait()

    def matrix_segment(src, dst, sem, t):
        nct, pieces, end = src.shape[1] // 128, [], t + SEG
        while t < end:
            band, c = divmod(t, nct)
            n = min(nct - c, end - t)
            pieces.append(functools.partial(copy, src, dst, (_band(8 * band), pl.ds(128 * c, 128 * n)),
                                            sem + (c // SEG if src is wq else 0)))
            t += n
        return pieces

    lead = range(ROW, ROW + ROW // 2, SEG)
    segments = [matrix_segment(wq, wq_b, S_WQ, t) for t in lead]
    for parity in range(2):
        for t in range(0, ROW, SEG):
            for src, dst, sem, turn in ((wq, wq_b, S_WQ, 0), (wg, wg_b, S_WG, WG_TURN[parity]),
                                        (wu, wu_b, S_WU, WU_TURN[parity])):
                size = src.shape[0] * src.shape[1] // TILE
                segments += [matrix_segment(src, dst, sem, r + (t + SEG * turn) % min(ROW, size - r))
                             for r in range(parity * ROW, size - t, 2 * ROW)
                             if not (src is wq and r + t in lead)]
    first = [(pc, int(i % 3 > 0)) for i, seg in enumerate(segments) for pc in seg]

    def cache_pieces(u):
        def piece(src, buf, sem, rows, slot, slot_rows, j):
            return lambda: pltpu.make_async_copy(src.at[rows, pl.ds(SK - W + j * SC, SC)],
                                                 buf.at[slot, slot_rows, pl.ds(j * SC, SC)],
                                                 sems.at[sem + (RING + 1) * j + slot])

        pieces, blocks = [], list(range(W // SC))
        for src, buf, sem, shift, order in ((kT, k_b, S_K, K_SHIFT, K_ORDER), (vT, v_b, S_V, V_SHIFT, V_ORDER)):
            p, b0 = divmod(UNIT * u - shift + NP * PB, PB)
            here, there = (PR * (p % NP), _slot(p)), (PR * ((p + 1) % NP), _slot(p + 1))
            bands = []
            for b in order:
                over = b0 + b >= PB
                base, slot = (_select(over, y, x) for x, y in zip(here, there))
                off = 8 * _select(over, b0 + b - PB, b0 + b)
                bands.append((_band(base + off), slot, _band(off)))
            pieces += [piece(src, buf, sem, *band, j) for half in range(2)
                       for j in (blocks[::-1] if half else blocks)
                       for band in bands[UNIT // 2 * half:UNIT // 2 * (half + 1)]]
        return [(pc, int(i % 4 > 0)) for i, pc in enumerate(pieces)]

    def wo_piece(r, t):
        return functools.partial(copy, wo, wo_b, (r, pl.ds(t // 2, SEG // 2)), S_WO + t // 16)

    def wd_piece(t, n, sem):
        return functools.partial(copy, wd, wd_b, pl.ds(t // 2, n // 2), sem)

    swept = [pc for t in range(0, ROW, SEG) for parity in range(2)
             for pc in [wo_piece(r, t) for r in WO_ORDER[parity]]
             + [wd_piece(r * ROW + (t + 16 * WD_TURN[parity]) % ROW, SEG, S_WD + t // 16)
                for r in range(parity, WD_ROWS, 2)]]
    last = [(pc, int(i % 4 > 0)) for i, pc in enumerate(swept)]
    solo = TAIL1 - 2 * LOOK
    last += [(wd_piece(t, 4, S_TAIL + (t - TAIL0) // 16), int(t % 32 >= 8)) for t in range(TAIL0, solo, 4)]
    last += [(wd_piece(t, 2, S_TAIL + (t - TAIL0) // 16), 1) for t in range(solo, TAIL1, 2)]

    def stream(cur, nxt, tasks):
        ahead = iter([pc for pc, queue in cur + nxt if queue == 1][LOOK:])
        for i, (pc, queue) in enumerate(cur):
            pc = next(ahead, None) if queue else pc
            if pc is not None:
                pc().start(priority=queue)
            for fn in tasks.get(i, ()):
                fn()

    st = {}
    small = [pltpu.make_async_copy(src, dst, sems.at[S_X + i])
             for i, (src, dst) in enumerate(((x_hbm, x_v), (gw_hbm, gw_v), (wr_hbm, wr_v)))]

    def gates():
        for c in small:
            c.wait()
        x = x_v[0].astype(f32)
        mix_s[0] = _fold(x, 8)
        for i, w in ((1, gw_v), (2, wr_v)):
            z = jnp.sum(x * w[...].astype(f32).reshape(1, D), axis=-1, keepdims=True)
            mix_s[i] = jnp.broadcast_to(jax.nn.sigmoid(z), (8, 128))

    def x_dot(w):
        return jnp.dot(jnp.broadcast_to(x_v[0], (8, D)), w, preferred_element_type=f32)

    def q_proj(j):
        idx = (slice(None), pl.ds(j * SC, SC))
        wait(wq_b, idx, S_WQ + j)
        q = x_dot(wq_b[idx])
        for m in range(SEG):
            q_s[j * SEG + m] = q[:, 128 * m:128 * (m + 1)]

    def gate_proj():
        wait(wg_b, ..., S_WG)
        t_s[...] = x_dot(wg_b[...])

    def up_proj():
        wait(wu_b, ..., S_WU)
        oh_s[O_ROWS:] = _fold(jax.nn.silu(t_s[...]) * x_dot(wu_b[...]), 16)

    def cache_block(buf, sem, p, j):
        idx = (_slot(p), slice(None), pl.ds(j * SC, SC))
        wait(buf, idx, sem + (RING + 1) * j + _slot(p))
        return buf[idx]

    def scores(p, j):
        q = jnp.concatenate([q_s[PR // 128 * p + m] for m in range(PR // 128)], axis=1)
        own = (_iota((8, PR), 1) >= DH) == (_iota((8, PR), 0) % 2 == 1)
        s_s[:, j * SC:(j + 1) * SC] = jnp.dot(jnp.where(own, q, 0.0).astype(bf16), cache_block(k_b, S_K, p, j),
                                              preferred_element_type=f32)

    def softmax():
        sc = s_s[...] * DH ** -0.5
        e = jnp.exp(sc - jnp.max(sc, axis=-1, keepdims=True))
        p_s[...] = e / jnp.sum(e, axis=-1, keepdims=True)

    def attend(p, j):
        o = jax.lax.dot_general(p_s[:, j * SC:(j + 1) * SC].astype(bf16), cache_block(v_b, S_V, p, j),
                                (((1,), (1,)), ((), ())), preferred_element_type=f32)
        o = o if j == 0 else t_s[:, :PR] + o
        if j < W // SC - 1:
            t_s[:, :PR] = o
        else:
            o = jnp.where(_iota((1, PR), 1) < DH, o[0:1], o[1:2])
            for m in range(PR // 128):
                oh_s[pl.ds(PR // 128 * p + m, 1)] = o[:, 128 * m:128 * (m + 1)]

    def expand():
        oh = oh_s[...].astype(bf16)
        src, lane = _iota((128, 128), 0), _iota((128, 128), 1)
        for s in range(CT):
            tile = 16 * s + lane // 8 - CT * (src // 8)
            sel = (tile >= 0) & (tile < CT) & (src % 8 == lane % 8)
            ex_s[s] = jnp.dot(oh, jnp.where(sel, 1.0, 0.0).astype(bf16), preferred_element_type=f32)
        lane, row = _iota((8, 128), 1), _iota((8, 128), 0)
        st['col'] = [(16 * s + lane // 8) % CT == row for s in range(CT)]
        st['a'] = st['y'] = jnp.zeros((8, 128), f32)
        picked = [jnp.where(lane == 8 * (b % 16) + row, oh_s[pl.ds(O_ROWS + b // 16, 1)], 0.0) for b in TAIL_BANDS]
        hb = jnp.dot(jnp.concatenate(picked, axis=0).astype(bf16), jnp.ones((128, 128), bf16),
                     preferred_element_type=f32)
        hb_s[...] = hb * ((1.0 - mix_s[1, 0:1]) * mix_s[2, 0:1])

    def block_dot(v0, blk, w):
        a, s = divmod(blk, CT)
        lhs = jnp.where(st['col'][s], ex_s[s, pl.ds(v0 + a, 1)], 0.0).astype(bf16)
        return jnp.dot(lhs, w.reshape(128, 128), preferred_element_type=f32)

    def out_proj(g):
        wait(wo_b, (slice(None), pl.ds(8 * g, 8)), S_WO + g)
        down = [r * NG + (g + WD_TURN[r % 2]) % NG for r in range(WD_ROWS)]
        for blk in down:
            for t in range(16 * blk, 16 * (blk + 1), SEG):
                wd_piece(t, SEG, S_WD + g)().wait()
        for r in range(WO_ROWS):
            st['a'] = st['a'] + block_dot(0, r * NG + g, wo_b[r, pl.ds(8 * g, 8)])
        for blk in down:
            st['y'] = st['y'] + block_dot(O_ROWS, blk, wd_b[pl.ds(8 * blk, 8)])

    def spread(start, step, fns):
        return {start + n * step: [fn] for n, fn in enumerate(fns)}

    def each(fn, n, *args):
        return [functools.partial(fn, *args, j) for j in range(n)]

    def attention(p):
        return each(scores, W // SC, p) + [softmax] + each(attend, W // SC, p)

    n_steps, shift = NP * PB // UNIT, max(K_SHIFT, V_SHIFT)

    def step(u, carry):
        p, b0 = divmod(UNIT * u - shift + PB, PB)
        tasks = spread(20, 24, [functools.partial(pl.when((b0 < UNIT) & (p >= 2)), fn) for fn in attention(p - 2)])
        tasks |= spread(21, 27, [functools.partial(pl.when(u == 1), fn)
                                 for fn in each(q_proj, H * DH // SC) + [gate_proj, up_proj]])
        cur = cache_pieces(u)
        stream(cur[:-40], cur[-40:], tasks)
        pl.when(u < n_steps - 1)(lambda: stream(cur[-40:], cache_pieces(u + 1), {}))
        return carry

    first[0][0]().start(priority=0)
    for pc in [pc for pc, queue in first if queue == 1][:LOOK]:
        pc().start(priority=1)
    stream(first[1:], cache_pieces(0), {41: [c.start for c in small], 200: [gates]})
    jax.lax.fori_loop(0, n_steps, step, 0)
    stream(cache_pieces(n_steps - 1)[-40:], last, {})

    done = (UNIT * (n_steps - 1) - shift) // PB
    tasks = spread(10, 18, [fn for p in range(done, NP) for fn in attention(p)] + [expand])
    pos = max(tasks)
    for g in range(NG):
        pos = min(max(pos + 12, len(swept) // NG * (g + 1) + 90), len(last) - 1)
        tasks.setdefault(pos, []).append(functools.partial(out_proj, g))
    stream(last, [], tasks)

    x, gate, rsel = mix_s[0], mix_s[1], mix_s[2]
    mixed = gate * st['a'] + (1.0 - gate) * (x + (x * 0.0 + st['y'] * rsel))
    acc = [jnp.where(_iota((8, 128), 0) == m, mixed, 0.0) for m in range(CT)]
    for t in range(TAIL0, TAIL1, 2):
        if t % 16 == 0:
            wait(wd_b, pl.ds(t // 2, 8), S_TAIL + (t - TAIL0) // 16)
        w = wd_b[t // 2].astype(f32)
        for half in range(2):
            band, m = divmod(t + half, CT)
            acc[m] = acc[m] + w[8 * half:8 * half + 8] * hb_s[pl.ds(8 * (band - TAIL_BANDS[0]), 8)]
    out_ref[0] = jnp.concatenate([jnp.sum(v, axis=0, keepdims=True) for v in acc], axis=1).astype(bf16)


def _memory_order(w):
    r, c = w.shape
    return w.reshape(r // 8, 8, c // 128, 128).transpose(0, 2, 1, 3).reshape(-1, 16, 128)


@jax.jit
def pallas_gated_mix__sliding_block_cached__moe_arch_mod__decode_kernel(
        A_x, A_k_cache, A_v_cache, A_wq, A_wo, B_x, B_w_r, B_w_gate, B_w_up, B_w_down, gate_w):
    del B_x
    kT = jnp.swapaxes(A_k_cache, 2, 3).reshape(H * DH, SK)
    vT = jnp.swapaxes(A_v_cache, 2, 3).reshape(H * DH, SK)
    wo = _memory_order(A_wo).reshape(WO_ROWS, ROW // 2, 16, 128)
    wd = _memory_order(B_w_down)
    vmem = pltpu.VMEM
    return pl.pallas_call(
        _kernel,
        out_shape=jax.ShapeDtypeStruct((1, 1, D), bf16),
        in_specs=[pl.BlockSpec(memory_space=pl.ANY)] * 10,
        out_specs=pl.BlockSpec(memory_space=pltpu.VMEM),
        scratch_shapes=[
            vmem((1, 1, D), bf16), vmem((D,), bf16), vmem((D,), bf16),
            vmem((D, H * DH), bf16), vmem((RING + 1, PR, W), bf16), vmem((RING + 1, PR, W), bf16),
            vmem(wo.shape, bf16), vmem((D, F), bf16), vmem((D, F), bf16), vmem(wd.shape, bf16),
            vmem((O_ROWS, 8, 128), f32), vmem((O_ROWS + 16, 128), f32), vmem((CT, O_ROWS + 16, 128), f32),
            vmem((8 * len(TAIL_BANDS), 128), f32), vmem((3, 8, 128), f32),
            vmem((8, W), f32), vmem((8, W), f32), vmem((8, F), f32),
            pltpu.SemaphoreType.DMA((N_SEMS,)),
        ],
        compiler_params=pltpu.CompilerParams(
            vmem_limit_bytes=80 * 1024 * 1024,
            disable_bounds_checks=True,
            disable_semaphore_checks=True,
        ),
        name="gated_mix_decode",
    )(A_x, kT, vT, A_wq, wo, B_w_r, B_w_gate, B_w_up, wd, gate_w)
```
